```python
import jax
import jax.numpy as jnp

def _softmax(x, axis=-1):
    return jax.nn.softmax(x, axis=axis)
def _gelu(x):
    return jax.nn.gelu(x, approximate=True)
def _silu(x):
    return jax.nn.silu(x)
def _sigmoid(x):
    return jax.nn.sigmoid(x)
def _layernorm(x, axis=-1, eps=1e-5):
    m = jnp.mean(x, axis=axis, keepdims=True)
    v = jnp.var(x, axis=axis, keepdims=True)
    return (x - m) / jnp.sqrt(v + eps)
def _scatter_add(tgt, idx, src, axis=0):
    return tgt.at[idx].add(src)
def _segment_sum(src, seg, n):
    return jax.ops.segment_sum(src, seg, n)
class _Rng:
    def __init__(self, key):
        self._k = key
    def _next(self):
        self._k, sub = jax.random.split(self._k)
        return sub
    def normal(self, shape):
        return jax.random.normal(self._next(), shape, dtype=jnp.bfloat16)
    def randint(self, lo, hi, shape):
        return jax.random.randint(self._next(), shape, lo, hi, dtype=jnp.int32)
    def uniform(self, shape, lo=0.0, hi=1.0):
        return jax.random.uniform(self._next(), shape, jnp.bfloat16, lo, hi)
    def permutation(self, n):
        return jax.random.permutation(self._next(), n)


kernel_name = 'interleave_layers__gqa_block_cached__sliding_block_cached__decode'

def _fwd_setup_inputs():
    _rng = _Rng(jax.random.key(int.from_bytes(__import__("os").urandom(4), "little")))
    _w = (lambda a: (lambda t: t.astype(jnp.bfloat16) if jnp.issubdtype(t.dtype, jnp.floating) else t)(jnp.asarray(a)))
    def _A_setup():
        B, Sq, D = 1, 1, 640
        Hq, Hkv, Sk, Dh = 32, 32, 8192, 128
        assert Hq % Hkv == 0, (Hq, Hkv)
        return {
            "x": _w((lambda *s: _rng.normal(s) * 0.05)(B, Sq, D)),
            "k_cache": _w((lambda *s: _rng.normal(s) * 0.05)(B, Hkv, Sk, Dh)),
            "v_cache": _w((lambda *s: _rng.normal(s) * 0.05)(B, Hkv, Sk, Dh)),
            "wq": _w((lambda *s: _rng.normal(s) * 0.05)(D, Hq * Dh) * (D ** -0.5)),
            "wo": _w((lambda *s: _rng.normal(s) * 0.05)(Hq * Dh, D) * ((Hq * Dh) ** -0.5)),
        }
    _A_in = _A_setup()

    def _B_setup():
        B, Sq, D = 1, 1, 640
        Hq, Hkv, Sk, Dh = 32, 32, 8192, 128
        assert Hq % Hkv == 0, (Hq, Hkv)
        return {
            "x": _w((lambda *s: _rng.normal(s) * 0.05)(B, Sq, D)),
            "k_cache": _w((lambda *s: _rng.normal(s) * 0.05)(B, Hkv, Sk, Dh)),
            "v_cache": _w((lambda *s: _rng.normal(s) * 0.05)(B, Hkv, Sk, Dh)),
            "wq": _w((lambda *s: _rng.normal(s) * 0.05)(D, Hq * Dh) * (D ** -0.5)),
            "wo": _w((lambda *s: _rng.normal(s) * 0.05)(Hq * Dh, D) * ((Hq * Dh) ** -0.5)),
        }
    _B_in = _B_setup()

    return {
        "A_x": _A_in["x"],
        "A_k_cache": _A_in["k_cache"],
        "A_v_cache": _A_in["v_cache"],
        "A_wq": _A_in["wq"],
        "A_wo": _A_in["wo"],
        "B_x": _B_in["x"],
        "B_k_cache": _B_in["k_cache"],
        "B_v_cache": _B_in["v_cache"],
        "B_wq": _B_in["wq"],
        "B_wo": _B_in["wo"],
    }

def _fwd_reference(A_x, A_k_cache, A_v_cache, A_wq, A_wo, B_x, B_k_cache, B_v_cache, B_wq, B_wo):
    def _A_ref(x, k_cache, v_cache, wq, wo):
        B, Sq, D = x.shape
        Hq, Dh = 32, 128
        Hkv = k_cache.shape[1]
        rep = Hq // Hkv
        q = (lambda x, *d: x.transpose(*d))((x @ wq).reshape(B, Sq, Hq, Dh), 0, 2, 1, 3)
        k = jnp.repeat(k_cache, rep, axis=1)
        v = jnp.repeat(v_cache, rep, axis=1)
        scores = jnp.einsum("bhqd,bhkd->bhqk", q, k) * (Dh ** -0.5)
        p = _softmax(scores, axis=-1)
        o = jnp.einsum("bhqk,bhkd->bhqd", p, v)
        return (lambda x, *d: x.transpose(*d))(o, 0, 2, 1, 3).reshape(B, Sq, Hq * Dh) @ wo

    def _B_ref(x, k_cache, v_cache, wq, wo):
        B, Sq, D = x.shape
        Hq, Dh = 32, 128
        Hkv, Sk = k_cache.shape[1], k_cache.shape[2]
        W = min(4096, max(256, Sk // 4))
        rep = Hq // Hkv
        q = (lambda x, *d: x.transpose(*d))((x @ wq).reshape(B, Sq, Hq, Dh), 0, 2, 1, 3)
        k = jnp.repeat(k_cache[:, :, Sk - W:, :], rep, axis=1)
        v = jnp.repeat(v_cache[:, :, Sk - W:, :], rep, axis=1)
        scores = jnp.einsum("bhqd,bhkd->bhqk", q, k) * (Dh ** -0.5)
        p = _softmax(scores, axis=-1)
        o = jnp.einsum("bhqk,bhkd->bhqd", p, v)
        return (lambda x, *d: x.transpose(*d))(o, 0, 2, 1, 3).reshape(B, Sq, Hq * Dh) @ wo

    x = A_x
    x = x + _A_ref(_layernorm(x, axis=-1), A_k_cache, A_v_cache, A_wq, A_wo)
    x = x + _B_ref(_layernorm(x, axis=-1), B_k_cache, B_v_cache, B_wq, B_wo)
    x = x + _A_ref(_layernorm(x, axis=-1), A_k_cache, A_v_cache, A_wq, A_wo)
    x = x + _B_ref(_layernorm(x, axis=-1), B_k_cache, B_v_cache, B_wq, B_wo)
    return x


def setup_inputs():
    _inp = _fwd_setup_inputs()
    _gk = jax.random.fold_in(jax.random.key(int.from_bytes(__import__("os").urandom(4), "little")), 2**31 - 1)
    _shapes = [[1, 1, 640]]
    _dtypes = ['bfloat16']
    _gks = jax.random.split(_gk, len(_shapes))
    _gs = [jax.random.normal(k, s, dtype=jnp.dtype(d)) * 0.05 for k, s, d in zip(_gks, _shapes, _dtypes)]
    _inp["grad_out"] = _gs[0]
    return _inp

def reference(A_x, A_k_cache, A_v_cache, A_wq, A_wo, B_k_cache, B_v_cache, B_wq, B_wo, B_x, grad_out):
    _const = dict(B_x=B_x)
    def _f(*_d):
        return _fwd_reference(**{'A_x': _d[0], 'A_k_cache': _d[1], 'A_v_cache': _d[2], 'A_wq': _d[3], 'A_wo': _d[4], 'B_k_cache': _d[5], 'B_v_cache': _d[6], 'B_wq': _d[7], 'B_wo': _d[8], **_const})
    _out, _vjp = jax.vjp(_f, A_x, A_k_cache, A_v_cache, A_wq, A_wo, B_k_cache, B_v_cache, B_wq, B_wo)
    _grads = _vjp(grad_out)
    _out0 = jnp.asarray(_out)
    return (_out0, *[jnp.asarray(_g) for _g in _grads])
```

```python
import functools

import jax
import jax.numpy as jnp
from jax import lax
import jax.experimental.pallas as pl
import jax.experimental.pallas.tpu as pltpu

D = 640
H = 32
DH = 128
SK = 8192
WIN = 2048
CH = 2048
SCALE = DH ** -0.5
EPS = 1e-5

f32 = jnp.float32
bf16 = jnp.bfloat16
NT = (((1,), (1,)), ((), ()))
TN = (((0,), (0,)), ((), ()))

X0 = 128
RING0 = X0 + 16
Y0 = X0 + 64
E0 = Y0 + 16
NE = 1
C1_SLOTS = (E0 + NE, E0 + NE + 1)
P1_SLOT = E0 + NE + 2
NSLOT = E0 + NE + 3
C3_SLOTS = (X0, X0 + 2)
P3_SLOT = X0 + 1
AUX_SLOT = X0 + 3
AUX_P4 = 1024
AUX_DS4 = 1536
NSTAGE = 3
TB = 2

Q1, Q2, Q3, Q4, O1, O2, O3, O4 = range(8)
DO_LATE, DO_EARLY, DQ3, DQ4, DQ_EARLY = range(8, 13)
NVEC = 13
XN0, RS0, G1 = 0, 4, 8

WQ_UNITS = D // 32
WO_UNITS = 16
A1_UNITS = 8 * 64
B_UNITS = 8 * 16
A3_UNITS = 4 * 32
B4_UNITS = 6 * 16
ZG, ZR = 4, 128
ZPER = 1024 // (ZG * ZR)
Z_UNITS = 384
LOOK1 = 80
Z23 = 20
ZA = 5
SW3 = 26
R3 = 6
ZF = (12, 7, 12, 6, 12, 12, 12, 4, 8, 6, 6)


def _rows(n):
    return lax.broadcasted_iota(jnp.int32, (n, 128), 0)


def _add(xs):
    return functools.reduce(lambda a, b: a + b, xs)


def _diag(*tiles):
    r = _rows(8)
    blocks = []
    for c in range(8):
        parts = [jnp.where(r == c, t, 0.0) for t in tiles]
        blocks.append(parts[0] if len(parts) == 1 else jnp.concatenate(parts, axis=0))
    return jnp.concatenate(blocks, axis=1).astype(bf16)


def _undiag(x):
    r = _rows(8)
    out = x[:, :128]
    for c in range(1, 8):
        out = jnp.where(r == c, x[:, 128 * c:128 * (c + 1)], out)
    return out


def _total(x):
    return jnp.sum(jnp.sum(x, axis=0, keepdims=True), axis=1, keepdims=True)


def _softmax(s):
    m = jnp.max(jnp.max(s, axis=0, keepdims=True), axis=1, keepdims=True)
    e = jnp.exp(s - m)
    return e / _total(e)


def _softmax_bwd(p, dp):
    return p * (dp - _total(p * dp)) * SCALE


def _loop(lo, hi, body):
    def step(i, carry):
        body(i)
        return carry
    lax.fori_loop(lo, hi, step, 0)


def _kernel(x_hbm, ak, av, awq, awo, bk, bv, bwq, bwo, g_hbm,
            out_hbm, dx_hbm, dak, dav, dawq, dawo, dbk, dbv, dbwq, dbwo,
            pool, wqa, woa, wqb, wob, zbuf, hv, rows, pscr, p2, io,
            sem_a1, sem_b2, sem_a3, sem_b4, sem_w, sem_z, sem_st, sem_io):

    if 0:
        pool32 = pool.bitcast(jnp.uint32)

        def tile(slot, start, size):
            return pltpu.bitcast(pool32[slot, pl.ds(start // 2, size // 2), :], bf16)

        def put(slot, start, size, value):
            pool32[slot, pl.ds(start // 2, size // 2), :] = pltpu.bitcast(value, jnp.uint32)
    else:
        def tile(slot, start, size):
            return pool[slot, pl.ds(start, size), :]

        def put(slot, start, size, value):
            pool[slot, pl.ds(start, size), :] = value

    def copy(src, dst, sem):
        return pltpu.make_async_copy(src, dst, sem)

    def wait_for(ref, sem):
        copy(ref, ref, sem).wait()

    def wq_unit(hbm, buf, sem, k):
        for n in range(8):
            m, r = lax.div(k, 4), pl.ds(pl.multiple_of((k & 3) * 32 + (n // 2) * 8, 8), 8)
            copy(hbm.at[m, r, pl.ds((n % 2) * 2048, 2048)], buf.at[n % 2, m, r, :],
                 sem).start(priority=n % 2)

    def wo_unit(hbm, buf, sem, k):
        for n in range(8):
            r = pl.ds(pl.multiple_of((n % 2) * 512 + k * 32, 32), 32)
            copy(hbm.at[n // 2, r, :], buf.at[n // 2, r, :], sem).start(priority=n % 2)

    def a1_unit(k):
        grp, rb = k >> 6, k & 63
        src = pl.ds(pl.multiple_of(rb * 128, 128), 128)
        dst = pl.ds(pl.multiple_of((rb & 15) * 128, 128), 128)
        for j in range(4):
            h = 4 * grp + j
            off = 4 * j + (rb >> 4)
            copy(ak.at[0, h, src, :], pool.at[X0 + 16 * (grp & 3) + off, dst, :],
                 sem_a1.at[grp]).start(priority=0)
            copy(av.at[0, h, src, :], pool.at[16 * grp + off, dst, :],
                 sem_a1.at[grp]).start(priority=1)

    def b2_slots(grp):
        base = Y0 + 8 * (grp & 1)
        kept = jnp.where(grp == 5, E0, base)
        return [(kept if n < NE else base) + n for n in range(8)]

    def b4_slots(grp):
        base = jnp.where(grp == 0, X0 + 4, jnp.where(grp == 5, RING0, RING0 + 8 + 8 * grp))
        base = jnp.where(grp > 5, Y0 + 8 * (grp & 1), base)
        kept = jnp.where(grp == 5, E0, base)
        return [(kept if n < NE else base) + n for n in range(8)]

    def b_copy(grp, rb, slots, sems, n):
        src = pl.ds(pl.multiple_of(SK - WIN + rb * 128, 128), 128)
        dst = pl.ds(pl.multiple_of(rb * 128, 128), 128)
        copy((bk, bv)[n % 2].at[0, 4 * grp + n // 2, src, :],
             pool.at[slots[n], dst, :], sems.at[grp]).start(priority=n % 2)

    def b2_unit(k):
        slots = b2_slots(k >> 4)
        for n in range(8):
            b_copy(k >> 4, k & 15, slots, sem_b2, n)

    def b4_unit(k):
        slots = b4_slots(k >> 4)
        for n in range(8):
            b_copy(k >> 4, k & 15, slots, sem_b4, n)

    def b4_last_unit(k):
        for n in range(NE, 8):
            b_copy(5, k, [RING0 + m for m in range(8)], sem_b4, n)

    def a3_slot(grp):
        return RING0 + 16 * jnp.where(grp == 3, 0, grp)

    def a3_unit(k):
        grp, u = k >> 5, k & 31
        for n in range(8):
            rb = 2 * u + n // 4
            src = pl.ds(pl.multiple_of(rb * 128, 128), 128)
            dst = pl.ds(pl.multiple_of((rb & 15) * 128, 128), 128)
            copy(ak.at[0, 4 * grp + n % 4, src, :],
                 pool.at[a3_slot(grp) + 4 * (n % 4) + (u >> 3), dst, :],
                 sem_a3.at[grp]).start(priority=n % 2)

    ZMODE = 11

    def z_unit(sem, k):
        nh = H // ZG
        nr = (SK - WIN) // ZR
        for n in range(ZPER):
            kk = k * (ZPER // 2) + n // 2
            if ZMODE % 10 == 0:
                hb, rb = kk & (nh - 1), lax.shift_right_logical(kk, nh.bit_length() - 1)
            elif ZMODE % 10 == 1:
                hb, rb = lax.div(kk, nr), lax.rem(kk, nr)
            elif ZMODE % 10 == 2:
                hb, rb = lax.div(kk, nr), lax.rem(kk + (n % 2) * (nr // 2), nr)
            elif ZMODE % 10 == 3:
                hb, rb = (lax.div(kk, nr) + (n % 2) * (nh // 2)) & (nh - 1), lax.rem(kk, nr)
            heads = pl.ds(hb * ZG, ZG)
            r = pl.ds(pl.multiple_of(rb * ZR, ZR), ZR)
            prio = (n % 2, 0)[ZMODE // 10]
            copy(zbuf, (dbk, dbv)[n % 2].at[0, heads, r, :], sem).start(priority=prio)

    def issue(lo, hi, segments):
        base = 0
        for count, fn in segments:
            if isinstance(lo, int) and isinstance(hi, int):
                first, last = (min(max(v - base, 0), count) for v in (lo, hi))
                if first < last:
                    _loop(first, last, fn)
            else:
                _loop(jnp.clip(lo - base, 0, count), jnp.clip(hi - base, 0, count), fn)
            base += count

    def issue_z(lo, hi, phase=1):
        _loop(lo, hi, functools.partial(z_unit, sem_z.at[phase]))

    def wait_z(units, phase):
        _loop(0, units * ZPER, lambda _: wait_for(zbuf, sem_z.at[phase]))

    stream1 = [
        (A1_UNITS, a1_unit),
        (WO_UNITS, functools.partial(wo_unit, awo, woa, sem_w.at[1])),
        (WQ_UNITS, functools.partial(wq_unit, bwq, wqb, sem_w.at[2])),
        (WO_UNITS, functools.partial(wo_unit, bwo, wob, sem_w.at[3])),
        (16, b2_unit),
    ]
    z_first = Z23 + ZA * SW3
    stream3 = [
        (A3_UNITS, a3_unit),
        (B4_UNITS - 16, b4_unit),
        (16, b4_last_unit),
    ]

    assert R3 * (32 - SW3) >= 32
    def row(i):
        return rows[pl.ds(i, 1), :]

    def layernorm(x, l):
        xc = x - jnp.mean(x, axis=1, keepdims=True)
        rstd = 1.0 / jnp.sqrt(jnp.mean(xc * xc, axis=1, keepdims=True) + EPS)
        xn = xc * rstd
        rows[pl.ds(XN0 + l, 1), :] = xn
        rows[pl.ds(RS0 + l, 1), :] = jnp.broadcast_to(rstd, (1, D))
        return xn

    def layernorm_bwd(dxn, l):
        xn = row(XN0 + l)
        return row(RS0 + l) * (dxn - jnp.mean(dxn, axis=1, keepdims=True)
                               - xn * jnp.mean(dxn * xn, axis=1, keepdims=True))

    def heads8(i):
        return pl.ds(pl.multiple_of(i * 8, 8), 8)

    def wo_block(buf, i):
        return buf[i]

    def wq_cols(i):
        return pl.ds(pl.multiple_of((i & 1) * 1024, 1024), 1024)

    def wq_block(buf, i):
        return buf[i >> 1, :, :, wq_cols(i)].reshape(D, 1024)

    def to_heads(vec, dst, product):
        lhs = jnp.broadcast_to(vec, (8, D)).astype(bf16)

        def body(i):
            hv[dst, heads8(i), :] = _undiag(product(lhs, i))
        _loop(0, 4, body)

    def from_heads(src, product):
        acc = lax.fori_loop(
            0, 4, lambda i, acc: acc + product(_diag(hv[src, heads8(i), :]), i),
            jnp.zeros((8, D), f32))
        return jnp.sum(acc, axis=0, keepdims=True)

    def x_wq(vec, buf, dst):
        to_heads(vec, dst, lambda lhs, i: jnp.dot(lhs, wq_block(buf, i), preferred_element_type=f32))

    def x_wo_t(vec, buf, dst):
        to_heads(vec, dst, lambda lhs, i: lax.dot_general(
            lhs, wo_block(buf, i), NT, preferred_element_type=f32))

    def heads_wo(src, buf):
        return from_heads(src, lambda lhs, i: jnp.dot(
            lhs, wo_block(buf, i), preferred_element_type=f32))

    def heads_wq_t(src, buf):
        return from_heads(src, lambda lhs, i: lax.dot_general(
            lhs, wq_block(buf, i), NT, preferred_element_type=f32))

    def two_rows(a, b):
        return jnp.concatenate(
            [jnp.broadcast_to(row(a), (8, D)), jnp.broadcast_to(row(b), (8, D))],
            axis=0).astype(bf16)

    def dwq(buf, hbm, sem, xa, xb, qa, qb):
        xs = two_rows(XN0 + xa, XN0 + xb)

        def half(c):
            for e in range(2):
                rhs = _diag(hv[qa, heads8(2 * c + e), :], hv[qb, heads8(2 * c + e), :])
                for m in range(D // 128):
                    for n in range(4):
                        buf[c, m, :, pl.ds(1024 * e + 256 * n, 256)] = lax.dot_general(
                            xs[:, 128 * m:128 * (m + 1)], rhs[:, 256 * n:256 * (n + 1)], TN,
                            preferred_element_type=f32).astype(bf16)

            def send(k):
                r = pl.ds(pl.multiple_of(k * 8, 8), 8)
                copy(buf.at[c, :, r, :],
                     hbm.at[:, r, pl.ds(pl.multiple_of(c * 2048, 2048), 2048)], sem).start()
            _loop(0, 16, send)
        _loop(0, 2, half)

    def dwo(buf, hbm, sem, ga, gb, oa, ob):
        gs = two_rows(G1 + ga, G1 + gb)
        r8 = _rows(8)

        def part(c):
            for i in range(4):
                lhs = jnp.concatenate(
                    [jnp.where(r8 == c, hv[o, pl.ds(8 * i, 8), :], 0.0) for o in (oa, ob)],
                    axis=0).astype(bf16)
                buf[i, pl.ds(pl.multiple_of(128 * c, 128), 128), :] = lax.dot_general(
                    lhs, gs, TN, preferred_element_type=f32).astype(bf16)
            for n in range(4):
                r = pl.ds(pl.multiple_of(128 * c + 32 * n, 32), 32)
                copy(buf.at[:, r, :], hbm.at[:, r, :], sem).start()
        _loop(0, 8, part)

    def head_vec(i, h):
        return jnp.broadcast_to(hv[i, pl.ds(h, 1), :], (8, 128))

    def against_rows(lhs, slot):
        out = []
        for b in range(2):
            tiles = jnp.concatenate(
                [tile(slot, 1024 * b + 128 * c, 128) for c in range(8)], axis=1)
            out.append(lax.dot_general(lhs, tiles, NT, preferred_element_type=f32))
        return out

    def weighted_rows(w, slot):
        acc = _add([jnp.dot(_diag(w[8 * b:8 * b + 8]), tile(slot, 1024 * b, 1024),
                            preferred_element_type=f32) for b in range(2)])
        return jnp.sum(acc, axis=0, keepdims=True)

    def cov_rows(n):
        return pl.ds(pl.multiple_of((n & 15) * 128, 128), 128)

    def p_rows(h):
        return pl.ds(pl.multiple_of(h * 64, 64), 64)

    def a_head(h, n, kslot, q, o, c_slots, p_slot, issue_point):
        lhs = _diag(head_vec(q, h))
        s = jnp.concatenate(
            [blk for c in range(4) for blk in against_rows(lhs, kslot + c)], axis=0)
        pscr[...] = _softmax(s * SCALE)
        tot = jnp.zeros((128 + 16, 128), f32)
        kbar = jnp.zeros((128, 128), f32)
        for c in range(4):
            if c == 1:
                issue_point(0)
            for t in range(0, 16, TB):
                keys = pl.ds(128 * t, 128 * TB)
                pr = jnp.concatenate(
                    [pscr[pl.ds(16 * c + t + j, 1), :] for j in range(TB)], axis=1)
                a = tile(kslot + c, 128 * t, 128 * TB).T.astype(f32) * pr
                kbar = kbar + _add([a[:, 128 * j:128 * (j + 1)] for j in range(TB)])
                lhs2 = jnp.concatenate(
                    [a.astype(bf16), jnp.broadcast_to(pr, (16, 128 * TB)).astype(bf16)], axis=0)
                tot = tot + jnp.dot(lhs2, tile(4 * h + c, 128 * t, 128 * TB),
                                    preferred_element_type=f32)
        out = tot[128:129]
        hv[o, pl.ds(h, 1), :] = out
        cov = (tot[:128] - jnp.sum(kbar, axis=1, keepdims=True) * out) * SCALE
        pool[jnp.where(n < 16, c_slots[0], c_slots[1]), cov_rows(n), :] = cov.astype(bf16)
        issue_point(1)
        pool[p_slot, p_rows(h), :] = pscr[...].astype(bf16)

    def a_dq(do, dq, c_slots, shift):
        def body(i):
            lhs = _diag(hv[do, heads8(i), :])
            n0 = (8 * i + shift) & (H - 1)
            slot = jnp.where(n0 < 16, c_slots[0], c_slots[1])
            covs = jnp.concatenate(
                [pool[slot, cov_rows(n0 + c), :] for c in range(8)], axis=1)
            hv[dq, heads8(i), :] = lax.dot_general(lhs, covs, NT, preferred_element_type=f32)
        _loop(0, 4, body)

    def b_rows(base, h):
        return pl.ds(pl.multiple_of(base + 16 * h, 16), 16)

    def b_group(grp, slots, q, o, p_ref, p_base, midway):
        heads = [4 * grp + j for j in range(4)]
        s = [jnp.concatenate(against_rows(_diag(head_vec(q, h)), slots[2 * j]), axis=0)
             for j, h in enumerate(heads)]
        p = [_softmax(x * SCALE) for x in s]
        midway()
        for j, h in enumerate(heads):
            p_ref[b_rows(p_base, h), :] = p[j].astype(bf16)
        for j, h in enumerate(heads):
            hv[o, pl.ds(h, 1), :] = weighted_rows(p[j], slots[2 * j + 1])

    def b_group_bwd(grp, p, do, dq, keep, midway):
        slots = b4_slots(grp)
        heads = [4 * grp + j for j in range(4)]
        dp = [jnp.concatenate(against_rows(_diag(head_vec(do, h)), slots[2 * j + 1]), axis=0)
              for j, h in enumerate(heads)]
        ds = [_softmax_bwd(a.astype(f32), b) for a, b in zip(p, dp)]
        midway()
        for j, h in enumerate(heads):
            keep(j, h, ds[j].astype(bf16))
        for j, h in enumerate(heads):
            hv[dq, pl.ds(h, 1), :] = weighted_rows(ds[j], slots[2 * j])

    def stage_base(b):
        return jnp.where(b == 0, X0 + 12, RING0 + 4 + 4 * b)

    def wait_stage(b):
        wait_for(pool.at[pl.ds(stage_base(b), 4)], sem_st.at[b])

    def emit(s, hbm, grp, row0, coef_row, tiles, tile0, va, vb):
        b = lax.rem(s, NSTAGE)
        base = stage_base(b)
        pl.when(s >= NSTAGE)(lambda: wait_stage(b))
        col = lax.broadcasted_iota(jnp.int32, (128, 128), 1) & (tiles - 1)
        second = (_rows(128) & tiles) != 0
        for j in range(4):
            h = 4 * grp + j
            coef = pool[AUX_SLOT, pl.ds(coef_row + 128 * j, 128), :]
            vecs = jnp.where(second, hv[vb, pl.ds(h, 1), :], hv[va, pl.ds(h, 1), :]).astype(bf16)
            for t in range(0, 16, 2):
                lhs = jnp.concatenate(
                    [jnp.where(col == tile0 + t + u, coef, jnp.zeros_like(coef))
                     for u in range(2)], axis=0)
                put(base + j, 128 * t, 256, jnp.dot(
                    lhs, vecs, preferred_element_type=f32).astype(bf16))
        ER = 128
        for r in range(CH // ER):
            copy(pool.at[pl.ds(base, 4), pl.ds(ER * r, ER), :],
                 hbm.at[0, pl.ds(4 * grp, 4), pl.ds(pl.multiple_of(row0 + ER * r, ER), ER), :],
                 sem_st.at[b]).start()

    x_in = copy(x_hbm, io.at[0], sem_io.at[0])
    g_in = copy(g_hbm, io.at[1], sem_io.at[1])
    x_in.start()
    g_in.start()
    _loop(0, WQ_UNITS, functools.partial(wq_unit, awq, wqa, sem_w.at[0]))
    _loop(0, LOOK1, a1_unit)
    zbuf[...] = jnp.zeros(zbuf.shape, bf16)
    x_in.wait()
    g_in.wait()
    x = io[0, 0].astype(f32)
    rows[pl.ds(G1 + 3, 1), :] = io[1, 0].astype(f32)

    wait_for(wqa, sem_w.at[0])
    x_wq(layernorm(x, 0), wqa, Q1)

    def layer1(h):
        grp = h >> 2
        kbase = X0 + 16 * (grp & 3)

        @pl.when((h & 3) == 0)
        def _():
            wait_for(pool.at[pl.ds(kbase, 16)], sem_a1.at[grp])
            wait_for(pool.at[pl.ds(16 * grp, 16)], sem_a1.at[grp])

        def point(i):
            lo = LOOK1 + 16 * h + 8 * i
            issue(lo, lo + 8, stream1)
        a_head(h, h, kbase + 4 * (h & 3), Q1, O1, C1_SLOTS, P1_SLOT, point)
    _loop(0, H, layer1)
    issue(LOOK1 + 16 * H, sum(n for n, _ in stream1), stream1)
    _loop(16, 24, b2_unit)

    wait_for(woa, sem_w.at[1])
    x = x + heads_wo(O1, woa)
    wait_for(wqb, sem_w.at[2])
    x_wq(layernorm(x, 1), wqb, Q2)

    def layer2(grp):
        stream2 = [(B_UNITS, b2_unit)]
        issue(jnp.maximum(16 * grp + 16, 24), 16 * grp + 26, stream2)
        slots = b2_slots(grp)
        for n in range(8):
            wait_for(pool.at[slots[n]], sem_b2.at[grp])
        issue_z(0, jnp.where(grp == 7, Z23 // 2, 0), 0)
        b_group(grp, slots, Q2, O2, p2, 0,
                lambda: issue(16 * grp + 26, 16 * grp + 32, stream2))
    _loop(0, 8, layer2)

    issue_z(Z23 // 2, Z23, 0)
    wait_for(wob, sem_w.at[3])
    x = x + heads_wo(O2, wob)
    x_wq(layernorm(x, 2), wqa, Q3)

    def layer3(n):
        h = (n + 16) & (H - 1)
        grp = h >> 2
        kbase = jnp.where(n < 16, X0 + 16 * (grp & 3), a3_slot(grp))

        @pl.when((n >= 16) & ((n & 3) == 0))
        def _():
            wait_for(pool.at[pl.ds(kbase, 16)], sem_a3.at[grp])

        def point(i):
            m = 2 * n + i
            issue_z(Z23 + ZA * jnp.minimum(m, SW3), Z23 + ZA * jnp.minimum(m + 1, SW3), 0)
            wait_z(jnp.where(m == SW3, z_first, 0), 0)
            issue(R3 * (m - SW3), R3 * (m + 1 - SW3), stream3)
        a_head(h, n, kbase + 4 * (h & 3), Q3, O3, C3_SLOTS, P3_SLOT, point)
    _loop(0, H, layer3)
    issue(R3 * (2 * H - SW3), sum(n for n, _ in stream3), stream3)
    for grp in range(6):
        slots = b4_slots(grp)
        for m in range(NE if grp == 5 else 0, 8):
            wait_for(pool.at[slots[m]], sem_b4.at[grp])

    z_at = [z_first]

    def fill(units):
        lo = z_at[0]
        z_at[0] = lo + units
        assert z_at[0] <= Z_UNITS
        if units:
            issue_z(lo, z_at[0])

    def fill_per_step(steps, units):
        lo = z_at[0]
        z_at[0] = lo + steps * units
        assert z_at[0] <= Z_UNITS
        return lambda i: issue_z(lo + units * i, lo + units * (i + 1)) if units else None
    z_spare = Z_UNITS - z_first - sum(ZF) - 7 * (ZF[1] + ZF[3] + ZF[7])
    assert z_spare >= 0, z_spare

    fill(ZF[0])
    x = x + heads_wo(O3, woa)
    x_wq(layernorm(x, 3), wqb, Q4)
    fill4 = fill_per_step(8, ZF[1])

    def layer4(n):
        grp = (n + 6) & 7
        slots = b4_slots(grp)
        b_group(grp, slots, Q4, O4, pool.at[AUX_SLOT], AUX_P4, lambda: fill4(n))
    _loop(0, 8, layer4)

    fill(ZF[2])
    io[2, 0] = (x + heads_wo(O4, wob)).astype(bf16)
    y_out = copy(io.at[2], out_hbm, sem_io.at[2])
    y_out.start()

    x_wo_t(row(G1 + 3), wob, DO_LATE)
    fill4b = fill_per_step(8, ZF[3])

    def layer4_bwd(grp):
        heads = [4 * grp + j for j in range(4)]

        def keep(j, h, ds):
            pool[AUX_SLOT, b_rows(AUX_DS4, h), :] = ds
        b_group_bwd(grp, [pool[AUX_SLOT, b_rows(AUX_P4, h), :] for h in heads],
                    DO_LATE, DQ4, keep, lambda: fill4b(grp))
    _loop(0, 8, layer4_bwd)

    fill(ZF[4])
    g = row(G1 + 3) + layernorm_bwd(heads_wq_t(DQ4, wqb), 3)
    rows[pl.ds(G1 + 2, 1), :] = g
    x_wo_t(g, woa, DO_EARLY)
    fill(ZF[5])
    a_dq(DO_EARLY, DQ3, C3_SLOTS, 16)
    g = g + layernorm_bwd(heads_wq_t(DQ3, wqa), 2)
    rows[pl.ds(G1 + 1, 1), :] = g

    fill(ZF[6] + z_spare)
    x_wo_t(g, wob, DO_EARLY)
    dwo(wob, dbwo, sem_w.at[3], 1, 3, O2, O4)
    fill2 = fill_per_step(8, ZF[7])

    def layer2_bwd(grp):
        pad = jnp.zeros((96, 128), bf16)
        heads = [4 * grp + j for j in range(4)]
        p = [p2[b_rows(0, h), :] for h in heads]

        def keep(j, h, ds):
            pool[AUX_SLOT, pl.ds(128 * j, 128), :] = jnp.concatenate(
                [p[j], pool[AUX_SLOT, b_rows(AUX_P4, h), :], pad], axis=0).T
            pool[AUX_SLOT, pl.ds(512 + 128 * j, 128), :] = jnp.concatenate(
                [ds, pool[AUX_SLOT, b_rows(AUX_DS4, h), :], pad], axis=0).T
        b_group_bwd(grp, p, DO_EARLY, DQ_EARLY, keep, lambda: fill2(grp))
        emit(2 * grp, dbv, grp, SK - WIN, 0, 16, 0, DO_EARLY, DO_LATE)
        emit(2 * grp + 1, dbk, grp, SK - WIN, 512, 16, 0, Q2, Q4)
    _loop(0, 8, layer2_bwd)

    fill(ZF[8])
    g = g + layernorm_bwd(heads_wq_t(DQ_EARLY, wqb), 1)
    rows[pl.ds(G1, 1), :] = g
    dwq(wqb, dbwq, sem_w.at[2], 1, 3, DQ_EARLY, DQ4)

    fill(ZF[9])
    x_wo_t(row(G1 + 2), woa, DO_LATE)
    x_wo_t(g, woa, DO_EARLY)
    dwo(woa, dawo, sem_w.at[1], 0, 2, O1, O3)
    fill(ZF[10])
    a_dq(DO_EARLY, DQ_EARLY, C1_SLOTS, 0)
    io[3, 0] = (g + layernorm_bwd(heads_wq_t(DQ_EARLY, wqa), 0)).astype(bf16)
    dx_out = copy(io.at[3], dx_hbm, sem_io.at[3])
    dx_out.start()
    dwq(wqa, dawq, sem_w.at[0], 0, 2, DQ_EARLY, DQ3)
    assert z_at[0] == Z_UNITS

    def cache_grads(grp):
        def coefficients(j):
            h = 4 * grp + j
            lhs = _diag(head_vec(DO_EARLY, h), head_vec(DO_LATE, h))
            dp = [blk for c in range(4) for blk in against_rows(lhs, 4 * h + c)]
            p = [pool[slot, p_rows(h), :] for slot in (P1_SLOT, P3_SLOT)]
            ds = [_softmax_bwd(p[l].astype(f32),
                               jnp.concatenate([blk[8 * l:8 * l + 8] for blk in dp], axis=0))
                  for l in range(2)]
            r = pl.multiple_of(128 * j, 128)
            pool[AUX_SLOT, pl.ds(r, 128), :] = jnp.concatenate(p, axis=0).T
            pool[AUX_SLOT, pl.ds(512 + r, 128), :] = jnp.concatenate(ds, axis=0).astype(bf16).T
        _loop(0, 4, coefficients)

        def chunk(c):
            s = 16 + 8 * grp + 2 * c
            emit(s, dav, grp, CH * c, 0, 64, 16 * c, DO_EARLY, DO_LATE)
            emit(s + 1, dak, grp, CH * c, 512, 64, 16 * c, Q1, Q3)
        _loop(0, 4, chunk)
    _loop(0, 8, cache_grads)

    y_out.wait()
    dx_out.wait()
    wait_z(Z_UNITS - z_first, 1)
    for i, buf in enumerate((wqa, woa, wqb, wob)):
        wait_for(buf, sem_w.at[i])
    for b in range(NSTAGE):
        wait_stage(b)


@jax.jit
def pallas_interleave_layers__gqa_block_cached__sliding_block_cached__decode_kernel(
    A_x, A_k_cache, A_v_cache, A_wq, A_wo, B_x, B_k_cache, B_v_cache, B_wq, B_wo, grad_out,
):
    del B_x
    weights = (A_k_cache, A_v_cache, A_wq, A_wo, B_k_cache, B_v_cache, B_wq, B_wo)
    wq3, wo3 = (5, D // 5, H * DH), (4, H * DH // 4, D)
    views = [w.reshape(shape) for w, shape in zip(weights, (
        A_k_cache.shape, A_v_cache.shape, wq3, wo3, B_k_cache.shape, B_v_cache.shape, wq3, wo3))]
    hbm = pl.BlockSpec(memory_space=pl.ANY)
    dma = pltpu.SemaphoreType.DMA
    outs = pl.pallas_call(
        _kernel,
        out_shape=[jax.ShapeDtypeStruct(a.shape, a.dtype) for a in [A_x, A_x] + views],
        in_specs=[hbm] * 10,
        out_specs=[hbm] * 10,
        scratch_shapes=[
            pltpu.VMEM((NSLOT - 0, CH, DH), bf16),
            pltpu.VMEM((2, 5, 128, 2048), bf16),
            pltpu.VMEM(wo3, bf16),
            pltpu.VMEM((2, 5, 128, 2048), bf16),
            pltpu.VMEM(wo3, bf16),
            pltpu.VMEM((ZG, ZR, DH), bf16),
            pltpu.VMEM((NVEC, H, DH), f32),
            pltpu.VMEM((16, D), f32),
            pltpu.VMEM((64, 128), f32),
            pltpu.VMEM((H * 16, 128), bf16),
            pltpu.VMEM((4, 1, 1, D), bf16),
            dma((8,)), dma((8,)), dma((4,)), dma((8,)), dma((4,)), dma((2,)),
            dma((NSTAGE,)), dma((4,)),
        ],
        compiler_params=pltpu.CompilerParams(vmem_limit_bytes=128 * 1024 * 1024, disable_bounds_checks=True),
    )(A_x, *views, grad_out)
    return tuple(o.reshape(a.shape) for o, a in zip(outs, (A_x, A_x) + weights))
```

```python
import functools

import jax
import jax.numpy as jnp
from jax import lax
import jax.experimental.pallas as pl
import jax.experimental.pallas.tpu as pltpu

D = 640
H = 32
DH = 128
SK = 8192
WIN = 2048
CH = 2048
SCALE = DH ** -0.5
EPS = 1e-5

f32 = jnp.float32
bf16 = jnp.bfloat16
NT = (((1,), (1,)), ((), ()))
TN = (((0,), (0,)), ((), ()))

CACHE_VIEW = (2, 4, 4 * SK, DH)
WQ_VIEW = (5, D // 5, H * DH)
WO_VIEW = (4, H * DH // 4, D)

B_RING = 192
B_KEPT, N_KEPT = 208, 5
C1_SLOTS = (213, 214)
NSLOT = 215
C3_SLOTS = (0, 4)
P3_SLOT, P1_SLOT = 1, 3
B_REST = 5
AUX_SLOT = 96
AUX_P4, AUX_DS4 = 1024, 1536
P2_SLOT = 97
NSTAGE = 3

Q1, Q2, Q3, Q4, O1, O2, O3, O4, DO_LATE, DO_EARLY, DQ3, DQ4 = range(12)
NVEC = 12
DQ_EARLY = O2
PROB = DO_LATE
XN0, G1 = 0, 4

W_UNITS = 16
A_UNITS, B_UNITS = 64, 16
Z_UNITS, Z_ROWS = 384, 128
OVERLAP = 3
LOOK1 = 80
Z_LEAD, Z_STEP1 = 28, 5
SWITCH1, SWITCH2 = 27, 60
R_BURST, R_STEP = 8, 6
Z_STEP2 = 6
Z_FIRST = Z_LEAD + Z_STEP1 * SWITCH1


def _check_second_read():
    def started(m):
        return R_STEP * (m - SWITCH1) + R_BURST if m > SWITCH1 else 0

    for unit, heads in ((0, 2), (4, 4), (20, 12), (84, 20), (148, 22), (164, 24),
                        (180, 26), (196, 28)):
        point = min(m for m in range(2 * H) if started(m + 1) > unit)
        assert (point + 1) // 2 >= heads
    assert started(48) >= 84 and started(56) >= 148
    assert started(SWITCH2 + 1) >= 212


_check_second_read()


def _rows(n):
    return lax.broadcasted_iota(jnp.int32, (n, 128), 0)


def _add(xs):
    return functools.reduce(lambda a, b: a + b, xs)


def _diag(*tiles):
    r = _rows(8)
    blocks = []
    for c in range(8):
        parts = [jnp.where(r == c, t, 0.0) for t in tiles]
        blocks.append(parts[0] if len(parts) == 1 else jnp.concatenate(parts, axis=0))
    return jnp.concatenate(blocks, axis=1).astype(bf16)


def _undiag(x):
    r = _rows(8)
    out = x[:, :128]
    for c in range(1, 8):
        out = jnp.where(r == c, x[:, 128 * c:128 * (c + 1)], out)
    return out


def _pick(blocks, l):
    return jnp.concatenate([blk[8 * l:8 * l + 8] for blk in blocks], axis=0)


def _total(x):
    return jnp.sum(jnp.sum(x, axis=0, keepdims=True), axis=1, keepdims=True)


def _softmax(s):
    m = jnp.max(jnp.max(s, axis=0, keepdims=True), axis=1, keepdims=True)
    e = jnp.exp(s - m)
    return e / _total(e)


def _softmax_bwd(p, dp):
    return p * (dp - _total(p * dp)) * SCALE


def _loop(lo, hi, body):
    def step(i, carry):
        body(i)
        return carry
    lax.fori_loop(lo, hi, step, 0)


def _once_if(cond, body):
    _loop(0, jnp.where(cond, 1, 0), lambda _: body())


def _member(grp, j):
    return 16 * (grp >> 2) + 4 * j + (grp & 3)


def _group_rows(grp, start, size):
    return pl.ds(pl.multiple_of(SK * (grp & 3) + start, size), size)


def _kernel(x_hbm, ak, av, awq, awo, bk, bv, bwq, bwo, g_hbm,
            out_hbm, dx_hbm, dak, dav, dawq, dawo, dbk, dbv, dbwq, dbwo,
            pool, wqa, woa, wqb, wob, zbuf, hv, rows, rstds, io,
            sem_a1, sem_a3, sem_b2, sem_b4, sem_w, sem_z, sem_stage, sem_io):
    copy = pltpu.make_async_copy

    def wait_for(ref, sem):
        copy(ref, ref, sem).wait()

    def slots(first, count):
        return pool.at[pl.ds(first, count)]

    def wq_unit(hbm, buf, sem, k):
        r = pl.ds(pl.multiple_of(k * 8, 8), 8)
        for n in range(10):
            copy(hbm.at[n // 2, r, pl.ds((n % 2) * 2048, 2048)], buf.at[n % 2, n // 2, r, :],
                 sem).start(priority=n % 2)

    def wo_unit(hbm, buf, sem, k):
        for n in range(8):
            r = pl.ds(pl.multiple_of((n % 2) * 512 + ((k + n) & 15) * 32, 32), 32)
            copy(hbm.at[n // 2, r, :], buf.at[n // 2, r, :], sem).start(priority=n % 2)

    def a1_slots(grp):
        first = 32 * jnp.where(grp < 2, grp + 4, grp - 2)
        return first, first + 16

    def a3_slots(grp):
        k, v = a1_slots(grp)
        return jnp.where(grp < 2, 32 + 64 * grp, k), jnp.where(grp < 2, 64 + 64 * grp, v)

    def a_copies(k, firsts, sems):
        grp, rb = k >> 6, k & 63
        src = _group_rows(grp, rb * 128, 128)
        dst = pl.ds(pl.multiple_of((rb & 15) * 128, 128), 128)
        for j in range(4):
            for e, hbm in enumerate((ak, av)):
                copy(hbm.at[grp >> 2, j, src, :], pool.at[firsts[e] + 4 * j + (rb >> 4), dst, :],
                     sems[e]).start(priority=e)

    def a1_unit(k):
        a_copies(k, a1_slots(k >> 6), (sem_a1.at[k >> 6],) * 2)

    def a3_unit(k):
        a_copies(k, a3_slots(k >> 6), [sem_a3.at[2 * (k >> 6) + e] for e in range(2)])

    def b2_slots(grp):
        first = B_RING + 8 * (grp & 1)
        kept = jnp.where(grp == 5, B_KEPT, first)
        return [(kept if n < N_KEPT else first) + n for n in range(8)]

    def b4_slots(grp):
        first = jnp.where(grp == 0, 8, jnp.where(grp < 3, 152 + 8 * grp, 8 + 8 * grp))
        first = jnp.where(grp > 5, B_RING + 8 * (grp & 1), first)
        kept = jnp.where(grp == 5, B_KEPT, first)
        rest = jnp.where(grp == 5, B_REST - N_KEPT, first)
        return [(kept if n < N_KEPT else rest) + n for n in range(8)]

    def b_copy(grp, rb, n, slot, sem):
        src = _group_rows(grp, SK - WIN + rb * 128, 128)
        dst = pl.ds(pl.multiple_of(rb * 128, 128), 128)
        copy((bk, bv)[n % 2].at[grp >> 2, n // 2, src, :], pool.at[slot, dst, :],
             sem).start(priority=n % 2)

    def b2_unit(k):
        grp = k >> 4
        for n, slot in enumerate(b2_slots(grp)):
            sem = jnp.where(k >= 8 * B_UNITS - OVERLAP, 16, 2 * grp + (n >= N_KEPT))
            b_copy(grp, k & 15, n, slot, sem_b2.at[sem])

    def b4_unit(k):
        grp = k >> 4
        sem = jnp.where(k >= 5 * B_UNITS - OVERLAP, 6, grp)
        for n, slot in enumerate(b4_slots(grp)):
            b_copy(grp, k & 15, n, slot, sem_b4.at[sem])

    def b4_rest_unit(k):
        for r in range(4):
            for n in range(N_KEPT, 8):
                b_copy(5, 4 * k + r, n, B_REST - N_KEPT + n, sem_b4.at[5])

    def zero_copies(k):
        per_group = (SK - WIN) // Z_ROWS
        grp = lax.div(k, per_group)
        r = _group_rows(grp, lax.rem(k, per_group) * Z_ROWS, Z_ROWS)
        sem = sem_z.at[jnp.where(k < Z_FIRST - OVERLAP, 0, 1)]
        return [copy(zbuf, hbm.at[grp >> 2, :, r, :], sem) for hbm in (dbk, dbv)]

    def write_zeros(lo, hi):
        _loop(lo, hi, lambda k: [c.start(priority=e) for e, c in enumerate(zero_copies(k))])

    def wait_zeros(lo, hi):
        _loop(lo, hi, lambda k: [c.wait() for c in zero_copies(k)])

    def issue(lo, hi, segments):
        base = 0
        for count, unit in segments:
            _loop(jnp.clip(lo - base, 0, count), jnp.clip(hi - base, 0, count), unit)
            base += count

    first_read = [
        (8 * A_UNITS, a1_unit),
        (W_UNITS, functools.partial(wo_unit, awo, woa, sem_w.at[1])),
        (W_UNITS, functools.partial(wq_unit, bwq, wqb, sem_w.at[2])),
        (2 * B_UNITS, b2_unit),
    ]
    second_read = [
        (4, b4_rest_unit),
        (B_UNITS, b4_unit),
        (2 * A_UNITS, a3_unit),
        (4 * B_UNITS, lambda k: b4_unit(k + B_UNITS)),
    ]

    def row(i):
        return rows[pl.ds(i, 1), :]

    def layernorm(x, l):
        xc = x - jnp.mean(x, axis=1, keepdims=True)
        rstd = 1.0 / jnp.sqrt(jnp.mean(xc * xc, axis=1, keepdims=True) + EPS)
        xn = xc * rstd
        rows[pl.ds(XN0 + l, 1), :] = xn
        rstds[pl.ds(l, 1), :] = jnp.broadcast_to(rstd, (1, 128))
        return xn

    def layernorm_bwd(dxn, l):
        xn = row(XN0 + l)
        return rstds[pl.ds(l, 1), pl.ds(0, 1)] * (
            dxn - jnp.mean(dxn, axis=1, keepdims=True)
            - xn * jnp.mean(dxn * xn, axis=1, keepdims=True))

    def heads8(i):
        return pl.ds(pl.multiple_of(i * 8, 8), 8)

    def wq_block(buf, i):
        cols = pl.ds(pl.multiple_of((i & 1) * 1024, 1024), 1024)
        return buf[i >> 1, :, :, cols].reshape(D, 1024)

    def to_heads(vec, dst, product):
        lhs = jnp.broadcast_to(vec, (8, D)).astype(bf16)

        def body(i):
            hv[dst, heads8(i), :] = _undiag(product(lhs, i))
        _loop(0, 4, body)

    def from_heads(src, product):
        acc = lax.fori_loop(
            0, 4, lambda i, acc: acc + product(_diag(hv[src, heads8(i), :]), i),
            jnp.zeros((8, D), f32))
        return jnp.sum(acc, axis=0, keepdims=True)

    def x_wq(vec, buf, dst):
        to_heads(vec, dst, lambda lhs, i: jnp.dot(
            lhs, wq_block(buf, i), preferred_element_type=f32))

    def x_wo_t(vec, buf, dst):
        to_heads(vec, dst, lambda lhs, i: lax.dot_general(
            lhs, buf[i], NT, preferred_element_type=f32))

    def heads_wo(src, buf):
        return from_heads(src, lambda lhs, i: jnp.dot(
            lhs, buf[i], preferred_element_type=f32))

    def heads_wq_t(src, buf):
        return from_heads(src, lambda lhs, i: lax.dot_general(
            lhs, wq_block(buf, i), NT, preferred_element_type=f32))

    def two_rows(a, b):
        return jnp.concatenate(
            [jnp.broadcast_to(row(a), (8, D)), jnp.broadcast_to(row(b), (8, D))],
            axis=0).astype(bf16)

    def dwq(buf, hbm, sem, xa, xb, qa, qb):
        xs = two_rows(XN0 + xa, XN0 + xb)

        def half(c):
            for e in range(2):
                rhs = _diag(hv[qa, heads8(2 * c + e), :], hv[qb, heads8(2 * c + e), :])
                for m in range(D // 128):
                    for n in range(4):
                        buf[c, m, :, pl.ds(1024 * e + 256 * n, 256)] = lax.dot_general(
                            xs[:, 128 * m:128 * (m + 1)], rhs[:, 256 * n:256 * (n + 1)], TN,
                            preferred_element_type=f32).astype(bf16)

            def send(k):
                r = pl.ds(pl.multiple_of(k * 8, 8), 8)
                copy(buf.at[c, :, r, :],
                     hbm.at[:, r, pl.ds(pl.multiple_of(c * 2048, 2048), 2048)], sem).start()
            _loop(0, 16, send)
        _loop(0, 2, half)

    def dwo(buf, hbm, sem, ga, gb, oa, ob):
        gs = two_rows(G1 + ga, G1 + gb)
        r8 = _rows(8)

        def part(c):
            for i in range(4):
                lhs = jnp.concatenate(
                    [jnp.where(r8 == c, hv[o, pl.ds(8 * i, 8), :], 0.0) for o in (oa, ob)],
                    axis=0).astype(bf16)
                buf[i, pl.ds(pl.multiple_of(128 * c, 128), 128), :] = lax.dot_general(
                    lhs, gs, TN, preferred_element_type=f32).astype(bf16)
            for n in range(4):
                r = pl.ds(pl.multiple_of(128 * c + 32 * n, 32), 32)
                copy(buf.at[:, r, :], hbm.at[:, r, :], sem).start()
        _loop(0, 8, part)

    def head_vec(i, h):
        return jnp.broadcast_to(hv[i, pl.ds(h, 1), :], (8, 128))

    def tile(slot, start, size):
        return pool[slot, pl.ds(start, size), :]

    def against_rows(lhs, slot):
        out = []
        for b in range(2):
            tiles = jnp.concatenate(
                [tile(slot, 1024 * b + 128 * c, 128) for c in range(8)], axis=1)
            out.append(lax.dot_general(lhs, tiles, NT, preferred_element_type=f32))
        return out

    def weighted_rows(w, slot):
        acc = _add([jnp.dot(_diag(w[8 * b:8 * b + 8]), tile(slot, 1024 * b, 1024),
                            preferred_element_type=f32) for b in range(2)])
        return jnp.sum(acc, axis=0, keepdims=True)

    def cov_rows(h):
        return pl.ds(pl.multiple_of((h & 15) * 128, 128), 128)

    def p_rows(h):
        return pl.ds(pl.multiple_of(h * 64, 64), 64)

    def a_head(h, kslot, vslot, qs, o, c_slots, p_slots, issue_point):
        lhs = _diag(*[head_vec(q, h) for q in qs])
        s = [blk for c in range(4) for blk in against_rows(lhs, kslot + c)]
        p = [_softmax(_pick(s, l) * SCALE) for l in range(len(qs))]
        for l in range(len(qs)):
            hv[PROB + 2 * l] = p[l][:32]
            hv[PROB + 2 * l + 1] = p[l][32:]
        k_mean = _add([weighted_rows(p[0][16 * c:16 * c + 16], kslot + c) for c in range(4)])
        issue_point(0)
        acc = jnp.zeros((128 + 16, 128), f32)
        for c in range(4):
            for t in range(0, 16, 2):
                pr = jnp.concatenate(
                    [hv[PROB + c // 2, pl.ds(16 * (c % 2) + t + u, 1), :] for u in range(2)],
                    axis=1)
                kp = tile(kslot + c, 128 * t, 256).T.astype(f32) * pr
                lhs = jnp.concatenate(
                    [kp.astype(bf16), jnp.broadcast_to(pr, (16, 256)).astype(bf16)], axis=0)
                acc = acc + jnp.dot(lhs, tile(vslot + c, 128 * t, 256),
                                    preferred_element_type=f32)
        out = acc[128:129]
        hv[o, pl.ds(h, 1), :] = out
        cov = (acc[:128] - jnp.broadcast_to(k_mean, (128, 128)).T * out) * SCALE
        issue_point(1)
        pool[jnp.where(h < 16, *c_slots), cov_rows(h), :] = cov.astype(bf16)
        for l, slot in enumerate(p_slots):
            pool[slot, p_rows(h), :] = jnp.concatenate(
                [hv[PROB + 2 * l], hv[PROB + 2 * l + 1]], axis=0).astype(bf16)

    def a_dq(do, dq, c_slots):
        def body(i):
            slot = jnp.where(i < 2, *c_slots)
            covs = jnp.concatenate(
                [pool[slot, cov_rows(8 * i + c), :] for c in range(8)], axis=1)
            hv[dq, heads8(i), :] = lax.dot_general(
                _diag(hv[do, heads8(i), :]), covs, NT, preferred_element_type=f32)
        _loop(0, 4, body)

    def b_rows(base, h):
        return pl.ds(pl.multiple_of(base + 16 * h, 16), 16)

    def b_group(grp, chunks, qs, o, keep, issue_point):
        heads = [_member(grp, j) for j in range(4)]
        s = [against_rows(_diag(*[head_vec(q, h) for q in qs]), chunks[2 * j])
             for j, h in enumerate(heads)]
        p = [[_softmax(_pick(x, l) * SCALE) for l in range(len(qs))] for x in s]
        issue_point()
        for j, h in enumerate(heads):
            for (slot, base), x in zip(keep, p[j]):
                pool[slot, b_rows(base, h), :] = x.astype(bf16)
        for j, h in enumerate(heads):
            hv[o, pl.ds(h, 1), :] = weighted_rows(p[j][0], chunks[2 * j + 1])

    def b_group_bwd(grp, p, do, dq, keep, issue_point):
        chunks = b4_slots(grp)
        heads = [_member(grp, j) for j in range(4)]
        dp = [jnp.concatenate(against_rows(_diag(head_vec(do, h)), chunks[2 * j + 1]), axis=0)
              for j, h in enumerate(heads)]
        ds = [_softmax_bwd(a.astype(f32), b) for a, b in zip(p, dp)]
        issue_point()
        for j, h in enumerate(heads):
            keep(j, h, ds[j].astype(bf16))
        for j, h in enumerate(heads):
            hv[dq, pl.ds(h, 1), :] = weighted_rows(ds[j], chunks[2 * j])

    def stage_slot(b):
        return jnp.where(b == 1, 8, 104 + 28 * b)

    def wait_stage(b):
        wait_for(slots(stage_slot(b), 8), sem_stage.at[b])

    def coef_rows(e, j):
        return pl.ds(pl.multiple_of(512 * e + 128 * j, 128), 128)

    def emit(s, grp, row0, outs, tiles, tile0):
        b = lax.rem(s, NSTAGE)
        first = stage_slot(b)
        _once_if(s >= NSTAGE, lambda: wait_stage(b))
        col = lax.broadcasted_iota(jnp.int32, (128, 128), 1) & (tiles - 1)
        second = (_rows(128) & tiles) != 0
        for e, (_, va, vb) in enumerate(outs):
            for j in range(4):
                h = _member(grp, j)
                coef = pool[AUX_SLOT, coef_rows(e, j), :]
                vecs = jnp.where(second, hv[vb, pl.ds(h, 1), :],
                                 hv[va, pl.ds(h, 1), :]).astype(bf16)
                for t in range(0, 16, 2):
                    lhs = jnp.concatenate(
                        [jnp.where(col == tile0 + t + u, coef, jnp.zeros_like(coef))
                         for u in range(2)], axis=0)
                    pool[first + 4 * e + j, pl.ds(128 * t, 256), :] = jnp.dot(
                        lhs, vecs, preferred_element_type=f32).astype(bf16)
        for r in range(0, CH, 128):
            for e, (hbm, _, _) in enumerate(outs):
                copy(pool.at[pl.ds(first + 4 * e, 4), pl.ds(r, 128), :],
                     hbm.at[grp >> 2, :, _group_rows(grp, row0 + r, 128), :],
                     sem_stage.at[b]).start()

    x_in = copy(x_hbm, io.at[0], sem_io.at[0])
    g_in = copy(g_hbm, io.at[1], sem_io.at[1])
    x_in.start()
    g_in.start()
    _loop(0, W_UNITS, functools.partial(wq_unit, awq, wqa, sem_w.at[0]))
    _loop(0, LOOK1, a1_unit)
    zbuf[...] = jnp.zeros(zbuf.shape, bf16)
    x_in.wait()
    g_in.wait()
    x = io[0, 0].astype(f32)
    rows[pl.ds(G1 + 3, 1), :] = io[1, 0].astype(f32)

    wait_for(wqa, sem_w.at[0])
    x_wq(layernorm(x, 0), wqa, Q1)

    def layer1(n):
        grp, j = n >> 2, n & 3
        k, v = a1_slots(grp)
        pl.when(j == 0)(lambda: wait_for(slots(k, 32), sem_a1.at[grp]))

        def issue_point(i):
            m = 2 * n + i
            issue(*(LOOK1 + 8 * t - 2 * jnp.maximum(t - 56, 0) for t in (m, m + 1)), first_read)
        a_head(_member(grp, j), k + 4 * j, v + 4 * j, (Q1,), O1, C1_SLOTS, (), issue_point)
    _loop(0, H, layer1)
    assert LOOK1 + 16 * H - 16 >= sum(count for count, _ in first_read)

    wob_unit = functools.partial(wo_unit, bwo, wob, sem_w.at[3])
    wait_for(woa, sem_w.at[1])
    x = x + heads_wo(O1, woa)
    _loop(0, W_UNITS // 2, wob_unit)
    wait_for(wqb, sem_w.at[2])
    x_wq(layernorm(x, 1), wqb, Q2)
    _loop(W_UNITS // 2, W_UNITS, wob_unit)
    head_rows = pl.ds(0, CH - 128 * OVERLAP)
    tail_rows = pl.ds(CH - 128 * OVERLAP, 128 * OVERLAP)

    def layer2(grp):
        chunks = b2_slots(grp)

        def wait_chunks(r):
            wait_for(pool.at[pl.ds(chunks[0], N_KEPT), r, :], sem_b2.at[2 * grp])
            wait_for(pool.at[pl.ds(chunks[N_KEPT], 8 - N_KEPT), r, :], sem_b2.at[2 * grp + 1])

        def last_group():
            wait_chunks(head_rows)
            write_zeros(0, Z_LEAD // 2)
            wait_for(pool.at[pl.ds(B_RING + 8, 8), tail_rows, :], sem_b2.at[16])
        _once_if(grp < 7, lambda: wait_chunks(pl.ds(0, CH)))
        _once_if(grp == 7, last_group)
        b_group(grp, chunks, (Q2,), O2, (), lambda: None)
        issue(B_UNITS * (grp + 2), B_UNITS * (grp + 3), [(8 * B_UNITS, b2_unit)])
    _loop(0, 8, layer2)

    write_zeros(Z_LEAD // 2, Z_LEAD)
    wait_for(wob, sem_w.at[3])
    x = x + heads_wo(O2, wob)
    x_wq(layernorm(x, 2), wqa, Q3)

    def read_started(m):
        return jnp.where(m > SWITCH1, R_STEP * (m - SWITCH1) + R_BURST, 0)

    def wait_second_read():
        wait_for(slots(B_REST, 8 - N_KEPT), sem_b4.at[5])
        for grp, first in enumerate((8, 160, 168, 32)):
            wait_for(slots(first, 8), sem_b4.at[grp])
        wait_for(pool.at[pl.ds(40, 8), head_rows, :], sem_b4.at[4])

    def layer3(n):
        grp, j = ((n >> 2) + 2) & 7, n & 3
        k, v = a3_slots(grp)

        @pl.when((grp < 2) & (j == 0))
        def _():
            wait_for(slots(k, 16), sem_a3.at[2 * grp])
            wait_for(slots(v, 16), sem_a3.at[2 * grp + 1])

        def issue_point(i):
            m = 2 * n + i
            write_zeros(*(Z_LEAD + Z_STEP1 * jnp.minimum(t, SWITCH1) for t in (m, m + 1)))
            wait_zeros(0, jnp.where(m == SWITCH1, Z_FIRST - OVERLAP, 0))
            issue(read_started(m), read_started(m + 1), second_read)
            _once_if(m == SWITCH2, wait_second_read)
            write_zeros(*(Z_FIRST + Z_STEP2 * jnp.maximum(t - SWITCH2, 0) for t in (m, m + 1)))
        a_head(_member(grp, j), k + 4 * j, v + 4 * j, (Q3, Q1), O3, C3_SLOTS,
               (P3_SLOT, P1_SLOT), issue_point)
    _loop(0, H, layer3)
    wait_for(pool.at[pl.ds(40, 8), tail_rows, :], sem_b4.at[6])

    z_next = [Z_FIRST + Z_STEP2 * (2 * H - SWITCH2)]

    def zeros_per_step(steps, units):
        lo = z_next[0]
        z_next[0] = lo + steps * units
        return lambda i: write_zeros(lo + units * i, lo + units * (i + 1))

    def zeros(units):
        zeros_per_step(1, units)(0)

    zeros(10)
    x = x + heads_wo(O3, woa)
    x_wq(layernorm(x, 3), wqb, Q4)
    zeros4 = zeros_per_step(8, 6)
    _loop(0, 8, lambda grp: b_group(
        grp, b4_slots(grp), (Q4, Q2), O4, ((AUX_SLOT, AUX_P4), (P2_SLOT, 0)),
        lambda: zeros4(grp)))
    zeros(10)
    io[0, 0] = (x + heads_wo(O4, wob)).astype(bf16)
    y_out = copy(io.at[0], out_hbm, sem_io.at[0])
    y_out.start()

    x_wo_t(row(G1 + 3), wob, DO_LATE)
    zeros4b = zeros_per_step(8, 5)

    def layer4_bwd(grp):
        def keep(j, h, ds):
            pool[AUX_SLOT, b_rows(AUX_DS4, h), :] = ds
        p = [pool[AUX_SLOT, b_rows(AUX_P4, _member(grp, j)), :] for j in range(4)]
        b_group_bwd(grp, p, DO_LATE, DQ4, keep, lambda: zeros4b(grp))
    _loop(0, 8, layer4_bwd)

    zeros(9)
    g = row(G1 + 3) + layernorm_bwd(heads_wq_t(DQ4, wqb), 3)
    rows[pl.ds(G1 + 2, 1), :] = g
    x_wo_t(g, woa, DQ3)
    zeros(9)
    a_dq(DQ3, DQ3, C3_SLOTS)
    g = g + layernorm_bwd(heads_wq_t(DQ3, wqa), 2)
    rows[pl.ds(G1 + 1, 1), :] = g

    zeros(27)
    x_wo_t(g, wob, DO_EARLY)
    dwo(wob, dbwo, sem_w.at[3], 1, 3, O2, O4)
    zeros2b = zeros_per_step(8, 3)

    def layer2_bwd(grp):
        p = [pool[P2_SLOT, b_rows(0, _member(grp, j)), :] for j in range(4)]
        pad = jnp.zeros((96, 128), bf16)

        def keep(j, h, ds):
            pool[AUX_SLOT, coef_rows(0, j), :] = jnp.concatenate(
                [p[j], pool[AUX_SLOT, b_rows(AUX_P4, h), :], pad], axis=0).T
            pool[AUX_SLOT, coef_rows(1, j), :] = jnp.concatenate(
                [ds, pool[AUX_SLOT, b_rows(AUX_DS4, h), :], pad], axis=0).T
        b_group_bwd(grp, p, DO_EARLY, DQ_EARLY, keep, lambda: zeros2b(grp))
        emit(grp, grp, SK - WIN, ((dbv, DO_EARLY, DO_LATE), (dbk, Q2, Q4)), 16, 0)
    _loop(0, 8, layer2_bwd)

    zeros(8)
    g = g + layernorm_bwd(heads_wq_t(DQ_EARLY, wqb), 1)
    rows[pl.ds(G1, 1), :] = g
    dwq(wqb, dbwq, sem_w.at[2], 1, 3, DQ_EARLY, DQ4)

    zeros(6)
    x_wo_t(row(G1 + 2), woa, DO_LATE)
    x_wo_t(g, woa, DO_EARLY)
    dwo(woa, dawo, sem_w.at[1], 0, 2, O1, O3)
    zeros(6)
    assert z_next[0] == Z_UNITS
    a_dq(DO_EARLY, DQ_EARLY, C1_SLOTS)
    io[1, 0] = (g + layernorm_bwd(heads_wq_t(DQ_EARLY, wqa), 0)).astype(bf16)
    dx_out = copy(io.at[1], dx_hbm, sem_io.at[1])
    dx_out.start()
    dwq(wqa, dawq, sem_w.at[0], 0, 2, DQ_EARLY, DQ3)

    def cache_grads(grp):
        def coefficients(j):
            h = _member(grp, j)
            vslot = a3_slots(grp)[1] + 4 * j
            lhs = _diag(head_vec(DO_EARLY, h), head_vec(DO_LATE, h))
            dp = [blk for c in range(4) for blk in against_rows(lhs, vslot + c)]
            p = [pool[slot, p_rows(h), :] for slot in (P1_SLOT, P3_SLOT)]
            ds = [_softmax_bwd(p[l].astype(f32), _pick(dp, l)) for l in range(2)]
            pool[AUX_SLOT, coef_rows(0, j), :] = jnp.concatenate(p, axis=0).T
            pool[AUX_SLOT, coef_rows(1, j), :] = jnp.concatenate(ds, axis=0).astype(bf16).T
        _loop(0, 4, coefficients)
        _loop(0, 4, lambda c: emit(
            8 + 4 * grp + c, grp, CH * c, ((dav, DO_EARLY, DO_LATE), (dak, Q1, Q3)), 64, 16 * c))
    _loop(0, 8, cache_grads)

    y_out.wait()
    dx_out.wait()
    wait_zeros(Z_FIRST - OVERLAP, Z_UNITS)
    for i, buf in enumerate((wqa, woa, wqb, wob)):
        wait_for(buf, sem_w.at[i])
    for b in range(NSTAGE):
        wait_stage(b)


@jax.jit
def pallas_interleave_layers__gqa_block_cached__sliding_block_cached__decode_kernel(
    A_x: jax.Array,
    A_k_cache: jax.Array,
    A_v_cache: jax.Array,
    A_wq: jax.Array,
    A_wo: jax.Array,
    B_x: jax.Array,
    B_k_cache: jax.Array,
    B_v_cache: jax.Array,
    B_wq: jax.Array,
    B_wo: jax.Array,
    grad_out: jax.Array,
):
    del B_x
    weights = (A_k_cache, A_v_cache, A_wq, A_wo, B_k_cache, B_v_cache, B_wq, B_wo)
    views = [w.reshape(shape) for w, shape in
             zip(weights, (CACHE_VIEW, CACHE_VIEW, WQ_VIEW, WO_VIEW) * 2)]
    hbm = pl.BlockSpec(memory_space=pl.ANY)
    dma = pltpu.SemaphoreType.DMA
    outs = pl.pallas_call(
        _kernel,
        out_shape=[jax.ShapeDtypeStruct(a.shape, a.dtype) for a in [A_x, A_x] + views],
        in_specs=[hbm] * 10,
        out_specs=[hbm] * 10,
        scratch_shapes=[
            pltpu.VMEM((NSLOT, CH, DH), bf16),
            pltpu.VMEM((2, 5, D // 5, H * DH // 2), bf16),
            pltpu.VMEM(WO_VIEW, bf16),
            pltpu.VMEM((2, 5, D // 5, H * DH // 2), bf16),
            pltpu.VMEM(WO_VIEW, bf16),
            pltpu.VMEM((4, Z_ROWS, DH), bf16),
            pltpu.VMEM((NVEC, H, DH), f32),
            pltpu.VMEM((8, D), f32),
            pltpu.VMEM((8, 128), f32),
            pltpu.VMEM((2, 1, 1, D), bf16),
            dma((8,)), dma((4,)), dma((17,)), dma((7,)), dma((4,)), dma((2,)),
            dma((NSTAGE,)), dma((2,)),
        ],
        compiler_params=pltpu.CompilerParams(
            vmem_limit_bytes=128 * 1024 * 1024,
            disable_bounds_checks=True,
            disable_semaphore_checks=True,
        ),
    )(A_x, *views, grad_out)
    return tuple(o.reshape(a.shape) for o, a in zip(outs, (A_x, A_x) + weights))
```

```python
import functools

import jax
import jax.numpy as jnp
from jax import lax
import jax.experimental.pallas as pl
import jax.experimental.pallas.tpu as pltpu

D = 640
H = 32
DH = 128
SK = 8192
WIN = 2048
CH = 2048
SCALE = DH ** -0.5
EPS = 1e-5

f32 = jnp.float32
bf16 = jnp.bfloat16
NT = (((1,), (1,)), ((), ()))
TN = (((0,), (0,)), ((), ()))

CACHE_VIEW = (2, 4, 4 * SK, DH)
WQ_VIEW = (5, D // 5, H * DH)
WO_VIEW = (4, H * DH // 4, D)

B_RING = 192
B_KEPT, N_KEPT = 208, 5
C1_SLOTS = (213, 214)
NSLOT = 215
C3_SLOTS = (0, 4)
P3_SLOT, P1_SLOT = 1, 3
B_REST = 5
AUX_SLOT = 96
AUX_P4, AUX_DS4 = 1024, 1536
P2_SLOT = 97
NSTAGE = 3

Q1, Q2, Q3, Q4, O1, O2, O3, O4, DO_LATE, DO_EARLY, DQ3, DQ4 = range(12)
NVEC = 12
DQ_EARLY = O2
PROB = DO_LATE
XN0, G1 = 0, 4

W_UNITS = 16
A_UNITS, B_UNITS = 64, 16
RUN = 112
Z_UNITS, Z_ROWS = 256, 192
OVERLAP, Z_OVERLAP = 3, 2
LOOK1 = 80
Z_LEAD, Z_STEP1 = 28, 3
SWITCH1, SWITCH2 = 27, 60
R_BURST, R_STEP = 8, 6
Z_STEP2 = 4
Z_FIRST = Z_LEAD + Z_STEP1 * SWITCH1


def _check_second_read():
    def started(m):
        return R_STEP * (m - SWITCH1) + R_BURST if m > SWITCH1 else 0

    for unit, heads in ((0, 2), (4, 4), (20, 12), (84, 20), (148, 22), (164, 24),
                        (180, 26), (196, 28)):
        point = min(m for m in range(2 * H) if started(m + 1) > unit)
        assert (point + 1) // 2 >= heads
    assert started(48) >= 84 and started(56) >= 148
    assert started(SWITCH2 + 1) >= 212


_check_second_read()


def _rows(n):
    return lax.broadcasted_iota(jnp.int32, (n, 128), 0)


def _add(xs):
    return functools.reduce(lambda a, b: a + b, xs)


def _diag(*tiles):
    r = _rows(8)
    blocks = []
    for c in range(8):
        parts = [jnp.where(r == c, t, 0.0) for t in tiles]
        blocks.append(parts[0] if len(parts) == 1 else jnp.concatenate(parts, axis=0))
    return jnp.concatenate(blocks, axis=1).astype(bf16)


def _undiag(x):
    r = _rows(8)
    out = x[:, :128]
    for c in range(1, 8):
        out = jnp.where(r == c, x[:, 128 * c:128 * (c + 1)], out)
    return out


def _pick(blocks, l):
    return jnp.concatenate([blk[8 * l:8 * l + 8] for blk in blocks], axis=0)


def _total(x):
    return jnp.sum(jnp.sum(x, axis=0, keepdims=True), axis=1, keepdims=True)


def _softmax(s):
    m = jnp.max(jnp.max(s, axis=0, keepdims=True), axis=1, keepdims=True)
    e = jnp.exp(s - m)
    return e / _total(e)


def _softmax_bwd(p, dp):
    return p * (dp - _total(p * dp)) * SCALE


def _loop(lo, hi, body):
    def step(i, carry):
        body(i)
        return carry
    lax.fori_loop(lo, hi, step, 0)


def _once_if(cond, body):
    _loop(0, jnp.where(cond, 1, 0), lambda _: body())


def _member(grp, j):
    return 16 * (grp >> 2) + 4 * j + (grp & 3)


def _group_rows(grp, start, size):
    return pl.ds(pl.multiple_of(SK * (grp & 3) + start, 16), size)


def _kernel(x_hbm, ak, av, awq, awo, bk, bv, bwq, bwo, g_hbm,
            out_hbm, dx_hbm, dak, dav, dawq, dawo, dbk, dbv, dbwq, dbwo,
            pool, wqa, woa, wqb, wob, zbuf, hv, rows, rstds, io,
            sem_a1, sem_a3, sem_b2, sem_b4, sem_w, sem_z, sem_stage, sem_io):
    copy = pltpu.make_async_copy

    def wait_for(ref, sem):
        copy(ref, ref, sem).wait()

    def slots(first, count):
        return pool.at[pl.ds(first, count)]

    def wq_unit(hbm, buf, sem, k):
        r = pl.ds(pl.multiple_of(k * 8, 8), 8)
        for n in range(10):
            copy(hbm.at[n // 2, r, pl.ds((n % 2) * 2048, 2048)], buf.at[n % 2, n // 2, r, :],
                 sem).start(priority=n % 2)

    def wo_unit(hbm, buf, sem, k):
        for n in range(8):
            r = pl.ds(pl.multiple_of((n % 2) * 512 + ((k + n) & 15) * 32, 32), 32)
            copy(hbm.at[n // 2, r, :], buf.at[n // 2, r, :], sem).start(priority=n % 2)

    def a1_slots(grp):
        first = 32 * jnp.where(grp < 2, grp + 4, grp - 2)
        return first, first + 16

    def a3_slots(grp):
        k, v = a1_slots(grp)
        return jnp.where(grp < 2, 32 + 64 * grp, k), jnp.where(grp < 2, 64 + 64 * grp, v)

    def a_copies(k, firsts, sems):
        grp, rb = k >> 6, k & 63
        src = _group_rows(grp, rb * 128, 128)
        dst = pl.ds(pl.multiple_of((rb & 15) * 128, 128), 128)
        for j in range(4):
            for e, hbm in enumerate((ak, av)):
                copy(hbm.at[grp >> 2, j, src, :], pool.at[firsts[e] + 4 * j + (rb >> 4), dst, :],
                     sems[e]).start(priority=e)

    def a1_unit(k):
        a_copies(k, a1_slots(k >> 6), (sem_a1.at[k >> 6],) * 2)

    def a3_unit(k):
        a_copies(k, a3_slots(k >> 6), [sem_a3.at[2 * (k >> 6) + e] for e in range(2)])

    def b2_slots(grp):
        first = B_RING + 8 * (grp & 1)
        kept = jnp.where(grp == 5, B_KEPT, first)
        return [(kept if n < N_KEPT else first) + n for n in range(8)]

    def b4_slots(grp):
        first = jnp.where(grp == 0, 8, jnp.where(grp < 3, 152 + 8 * grp, 8 + 8 * grp))
        first = jnp.where(grp > 5, B_RING + 8 * (grp & 1), first)
        kept = jnp.where(grp == 5, B_KEPT, first)
        rest = jnp.where(grp == 5, B_REST - N_KEPT, first)
        return [(kept if n < N_KEPT else rest) + n for n in range(8)]

    def b_copy(grp, rb, n, slot, sem):
        src = _group_rows(grp, SK - WIN + rb * 128, 128)
        dst = pl.ds(pl.multiple_of(rb * 128, 128), 128)
        copy((bk, bv)[n % 2].at[grp >> 2, n // 2, src, :], pool.at[slot, dst, :],
             sem).start(priority=n % 2)

    def b2_unit(k):
        grp = k >> 4
        for n, slot in enumerate(b2_slots(grp)):
            sem = jnp.where(k >= 8 * B_UNITS - OVERLAP, 16, 2 * grp + (n >= N_KEPT))
            b_copy(grp, k & 15, n, slot, sem_b2.at[sem])

    def b4_unit(k):
        grp = k >> 4
        sem = jnp.where(k >= 5 * B_UNITS - OVERLAP, 6, grp)
        for n, slot in enumerate(b4_slots(grp)):
            b_copy(grp, k & 15, n, slot, sem_b4.at[sem])

    def b4_rest_unit(k):
        for r in range(4):
            for n in range(N_KEPT, 8):
                b_copy(5, 4 * k + r, n, B_REST - N_KEPT + n, sem_b4.at[5])

    def zero_copies(k):
        grp, first = k >> 5, (k & 31) * Z_ROWS
        sem = sem_z.at[jnp.where(k < Z_FIRST - Z_OVERLAP, 0, 1)]
        pieces = ((dbk, 0, RUN), (dbv, 0, Z_ROWS - RUN),
                  (dbk, RUN, Z_ROWS - RUN), (dbv, Z_ROWS - RUN, RUN))
        return [copy(zbuf.at[:, pl.ds(0, size), :],
                     hbm.at[grp >> 2, :, _group_rows(grp, first + r, size), :], sem)
                for hbm, r, size in pieces]

    def write_zeros(lo, hi):
        _loop(lo, hi, lambda k: [c.start() for c in zero_copies(k)])

    def wait_zeros(lo, hi):
        _loop(lo, hi, lambda k: [c.wait() for c in zero_copies(k)])

    def issue(lo, hi, segments):
        base = 0
        for count, unit in segments:
            _loop(jnp.clip(lo - base, 0, count), jnp.clip(hi - base, 0, count), unit)
            base += count

    first_read = [
        (8 * A_UNITS, a1_unit),
        (W_UNITS, functools.partial(wo_unit, awo, woa, sem_w.at[1])),
        (W_UNITS, functools.partial(wq_unit, bwq, wqb, sem_w.at[2])),
        (2 * B_UNITS, b2_unit),
    ]
    second_read = [
        (4, b4_rest_unit),
        (B_UNITS, b4_unit),
        (2 * A_UNITS, a3_unit),
        (4 * B_UNITS, lambda k: b4_unit(k + B_UNITS)),
    ]

    def row(i):
        return rows[pl.ds(i, 1), :]

    def layernorm(x, l):
        xc = x - jnp.mean(x, axis=1, keepdims=True)
        rstd = 1.0 / jnp.sqrt(jnp.mean(xc * xc, axis=1, keepdims=True) + EPS)
        xn = xc * rstd
        rows[pl.ds(XN0 + l, 1), :] = xn
        rstds[pl.ds(l, 1), :] = jnp.broadcast_to(rstd, (1, 128))
        return xn

    def layernorm_bwd(dxn, l):
        xn = row(XN0 + l)
        return rstds[pl.ds(l, 1), pl.ds(0, 1)] * (
            dxn - jnp.mean(dxn, axis=1, keepdims=True)
            - xn * jnp.mean(dxn * xn, axis=1, keepdims=True))

    def heads8(i):
        return pl.ds(pl.multiple_of(i * 8, 8), 8)

    def wq_block(buf, i):
        cols = pl.ds(pl.multiple_of((i & 1) * 1024, 1024), 1024)
        return buf[i >> 1, :, :, cols].reshape(D, 1024)

    def to_heads(vec, dst, product):
        lhs = jnp.broadcast_to(vec, (8, D)).astype(bf16)

        def body(i):
            hv[dst, heads8(i), :] = _undiag(product(lhs, i))
        _loop(0, 4, body)

    def from_heads(src, product):
        acc = lax.fori_loop(
            0, 4, lambda i, acc: acc + product(_diag(hv[src, heads8(i), :]), i),
            jnp.zeros((8, D), f32))
        return jnp.sum(acc, axis=0, keepdims=True)

    def x_wq(vec, buf, dst):
        to_heads(vec, dst, lambda lhs, i: jnp.dot(
            lhs, wq_block(buf, i), preferred_element_type=f32))

    def x_wo_t(vec, buf, dst):
        to_heads(vec, dst, lambda lhs, i: lax.dot_general(
            lhs, buf[i], NT, preferred_element_type=f32))

    def heads_wo(src, buf):
        return from_heads(src, lambda lhs, i: jnp.dot(
            lhs, buf[i], preferred_element_type=f32))

    def heads_wq_t(src, buf):
        return from_heads(src, lambda lhs, i: lax.dot_general(
            lhs, wq_block(buf, i), NT, preferred_element_type=f32))

    def two_rows(a, b):
        return jnp.concatenate(
            [jnp.broadcast_to(row(a), (8, D)), jnp.broadcast_to(row(b), (8, D))],
            axis=0).astype(bf16)

    def dwq(buf, hbm, sem, xa, xb, qa, qb):
        xs = two_rows(XN0 + xa, XN0 + xb)

        def half(c):
            for e in range(2):
                rhs = _diag(hv[qa, heads8(2 * c + e), :], hv[qb, heads8(2 * c + e), :])
                for m in range(D // 128):
                    for n in range(4):
                        buf[c, m, :, pl.ds(1024 * e + 256 * n, 256)] = lax.dot_general(
                            xs[:, 128 * m:128 * (m + 1)], rhs[:, 256 * n:256 * (n + 1)], TN,
                            preferred_element_type=f32).astype(bf16)

            def send(k):
                r = pl.ds(pl.multiple_of(k * 8, 8), 8)
                copy(buf.at[c, :, r, :],
                     hbm.at[:, r, pl.ds(pl.multiple_of(c * 2048, 2048), 2048)], sem).start()
            _loop(0, 16, send)
        _loop(0, 2, half)

    def dwo(buf, hbm, sem, ga, gb, oa, ob):
        gs = two_rows(G1 + ga, G1 + gb)
        r8 = _rows(8)

        def part(c):
            for i in range(4):
                lhs = jnp.concatenate(
                    [jnp.where(r8 == c, hv[o, pl.ds(8 * i, 8), :], 0.0) for o in (oa, ob)],
                    axis=0).astype(bf16)
                buf[i, pl.ds(pl.multiple_of(128 * c, 128), 128), :] = lax.dot_general(
                    lhs, gs, TN, preferred_element_type=f32).astype(bf16)
            for n in range(4):
                r = pl.ds(pl.multiple_of(128 * c + 32 * n, 32), 32)
                copy(buf.at[:, r, :], hbm.at[:, r, :], sem).start()
        _loop(0, 8, part)

    def head_vec(i, h):
        return jnp.broadcast_to(hv[i, pl.ds(h, 1), :], (8, 128))

    def tile(slot, start, size):
        return pool[slot, pl.ds(start, size), :]

    def against_rows(lhs, slot):
        out = []
        for b in range(2):
            tiles = jnp.concatenate(
                [tile(slot, 1024 * b + 128 * c, 128) for c in range(8)], axis=1)
            out.append(lax.dot_general(lhs, tiles, NT, preferred_element_type=f32))
        return out

    def weighted_rows(w, slot):
        acc = _add([jnp.dot(_diag(w[8 * b:8 * b + 8]), tile(slot, 1024 * b, 1024),
                            preferred_element_type=f32) for b in range(2)])
        return jnp.sum(acc, axis=0, keepdims=True)

    def cov_rows(h):
        return pl.ds(pl.multiple_of((h & 15) * 128, 128), 128)

    def p_rows(h):
        return pl.ds(pl.multiple_of(h * 64, 64), 64)

    def a_head(h, kslot, vslot, qs, o, c_slots, p_slots, issue_point):
        lhs = _diag(*[head_vec(q, h) for q in qs])
        s = [blk for c in range(4) for blk in against_rows(lhs, kslot + c)]
        p = [_softmax(_pick(s, l) * SCALE) for l in range(len(qs))]
        for l in range(len(qs)):
            hv[PROB + 2 * l] = p[l][:32]
            hv[PROB + 2 * l + 1] = p[l][32:]
        k_mean = _add([weighted_rows(p[0][16 * c:16 * c + 16], kslot + c) for c in range(4)])
        issue_point(0)
        acc = jnp.zeros((128 + 16, 128), f32)
        for c in range(4):
            for t in range(0, 16, 2):
                pr = jnp.concatenate(
                    [hv[PROB + c // 2, pl.ds(16 * (c % 2) + t + u, 1), :] for u in range(2)],
                    axis=1)
                kp = tile(kslot + c, 128 * t, 256).T.astype(f32) * pr
                lhs = jnp.concatenate(
                    [kp.astype(bf16), jnp.broadcast_to(pr, (16, 256)).astype(bf16)], axis=0)
                acc = acc + jnp.dot(lhs, tile(vslot + c, 128 * t, 256),
                                    preferred_element_type=f32)
        out = acc[128:129]
        hv[o, pl.ds(h, 1), :] = out
        cov = (acc[:128] - jnp.broadcast_to(k_mean, (128, 128)).T * out) * SCALE
        issue_point(1)
        pool[jnp.where(h < 16, *c_slots), cov_rows(h), :] = cov.astype(bf16)
        for l, slot in enumerate(p_slots):
            pool[slot, p_rows(h), :] = jnp.concatenate(
                [hv[PROB + 2 * l], hv[PROB + 2 * l + 1]], axis=0).astype(bf16)

    def a_dq(do, dq, c_slots):
        def body(i):
            slot = jnp.where(i < 2, *c_slots)
            covs = jnp.concatenate(
                [pool[slot, cov_rows(8 * i + c), :] for c in range(8)], axis=1)
            hv[dq, heads8(i), :] = lax.dot_general(
                _diag(hv[do, heads8(i), :]), covs, NT, preferred_element_type=f32)
        _loop(0, 4, body)

    def b_rows(base, h):
        return pl.ds(pl.multiple_of(base + 16 * h, 16), 16)

    def b_group(grp, chunks, qs, o, keep, issue_point):
        heads = [_member(grp, j) for j in range(4)]
        s = [against_rows(_diag(*[head_vec(q, h) for q in qs]), chunks[2 * j])
             for j, h in enumerate(heads)]
        p = [[_softmax(_pick(x, l) * SCALE) for l in range(len(qs))] for x in s]
        issue_point()
        for j, h in enumerate(heads):
            for (slot, base), x in zip(keep, p[j]):
                pool[slot, b_rows(base, h), :] = x.astype(bf16)
        for j, h in enumerate(heads):
            hv[o, pl.ds(h, 1), :] = weighted_rows(p[j][0], chunks[2 * j + 1])

    def b_group_bwd(grp, p, do, dq, keep, issue_point):
        chunks = b4_slots(grp)
        heads = [_member(grp, j) for j in range(4)]
        dp = [jnp.concatenate(against_rows(_diag(head_vec(do, h)), chunks[2 * j + 1]), axis=0)
              for j, h in enumerate(heads)]
        ds = [_softmax_bwd(a.astype(f32), b) for a, b in zip(p, dp)]
        issue_point()
        for j, h in enumerate(heads):
            keep(j, h, ds[j].astype(bf16))
        for j, h in enumerate(heads):
            hv[dq, pl.ds(h, 1), :] = weighted_rows(ds[j], chunks[2 * j])

    def stage_slot(b):
        return jnp.where(b == 1, 8, 104 + 28 * b)

    def wait_stage(b):
        wait_for(slots(stage_slot(b), 8), sem_stage.at[b])

    def coef_rows(e, j):
        return pl.ds(pl.multiple_of(512 * e + 128 * j, 128), 128)

    def emit(s, grp, row0, outs, tiles, tile0):
        b = lax.rem(s, NSTAGE)
        first = stage_slot(b)
        _once_if(s >= NSTAGE, lambda: wait_stage(b))
        col = lax.broadcasted_iota(jnp.int32, (128, 128), 1) & (tiles - 1)
        second = (_rows(128) & tiles) != 0
        for e, (_, va, vb) in enumerate(outs):
            for j in range(4):
                h = _member(grp, j)
                coef = pool[AUX_SLOT, coef_rows(e, j), :]
                vecs = jnp.where(second, hv[vb, pl.ds(h, 1), :],
                                 hv[va, pl.ds(h, 1), :]).astype(bf16)
                for t in range(0, 16, 2):
                    lhs = jnp.concatenate(
                        [jnp.where(col == tile0 + t + u, coef, jnp.zeros_like(coef))
                         for u in range(2)], axis=0)
                    pool[first + 4 * e + j, pl.ds(128 * t, 256), :] = jnp.dot(
                        lhs, vecs, preferred_element_type=f32).astype(bf16)
        for r in range(0, CH, RUN):
            size = min(RUN, CH - r)
            for e, (hbm, _, _) in enumerate(outs):
                copy(pool.at[pl.ds(first + 4 * e, 4), pl.ds(r, size), :],
                     hbm.at[grp >> 2, :, _group_rows(grp, row0 + r, size), :],
                     sem_stage.at[b]).start()

    x_in = copy(x_hbm, io.at[0], sem_io.at[0])
    g_in = copy(g_hbm, io.at[1], sem_io.at[1])
    x_in.start()
    g_in.start()
    _loop(0, W_UNITS, functools.partial(wq_unit, awq, wqa, sem_w.at[0]))
    _loop(0, LOOK1, a1_unit)
    zbuf[...] = jnp.zeros(zbuf.shape, bf16)
    x_in.wait()
    g_in.wait()
    x = io[0, 0].astype(f32)
    rows[pl.ds(G1 + 3, 1), :] = io[1, 0].astype(f32)

    wait_for(wqa, sem_w.at[0])
    x_wq(layernorm(x, 0), wqa, Q1)

    def layer1(n):
        grp, j = n >> 2, n & 3
        k, v = a1_slots(grp)
        pl.when(j == 0)(lambda: wait_for(slots(k, 32), sem_a1.at[grp]))

        def issue_point(i):
            m = 2 * n + i
            issue(*(LOOK1 + 8 * t - 2 * jnp.maximum(t - 56, 0) for t in (m, m + 1)), first_read)
        a_head(_member(grp, j), k + 4 * j, v + 4 * j, (Q1,), O1, C1_SLOTS, (), issue_point)
    _loop(0, H, layer1)
    assert LOOK1 + 16 * H - 16 >= sum(count for count, _ in first_read)

    wob_unit = functools.partial(wo_unit, bwo, wob, sem_w.at[3])
    wait_for(woa, sem_w.at[1])
    x = x + heads_wo(O1, woa)
    _loop(0, W_UNITS // 2, wob_unit)
    wait_for(wqb, sem_w.at[2])
    x_wq(layernorm(x, 1), wqb, Q2)
    _loop(W_UNITS // 2, W_UNITS, wob_unit)
    head_rows = pl.ds(0, CH - 128 * OVERLAP)
    tail_rows = pl.ds(CH - 128 * OVERLAP, 128 * OVERLAP)

    def layer2(grp):
        chunks = b2_slots(grp)

        def wait_chunks(r):
            wait_for(pool.at[pl.ds(chunks[0], N_KEPT), r, :], sem_b2.at[2 * grp])
            wait_for(pool.at[pl.ds(chunks[N_KEPT], 8 - N_KEPT), r, :], sem_b2.at[2 * grp + 1])

        def last_group():
            wait_chunks(head_rows)
            write_zeros(0, Z_LEAD // 2)
            wait_for(pool.at[pl.ds(B_RING + 8, 8), tail_rows, :], sem_b2.at[16])
        _once_if(grp < 7, lambda: wait_chunks(pl.ds(0, CH)))
        _once_if(grp == 7, last_group)
        b_group(grp, chunks, (Q2,), O2, (), lambda: None)
        issue(B_UNITS * (grp + 2), B_UNITS * (grp + 3), [(8 * B_UNITS, b2_unit)])
    _loop(0, 8, layer2)

    write_zeros(Z_LEAD // 2, Z_LEAD)
    wait_for(wob, sem_w.at[3])
    x = x + heads_wo(O2, wob)
    x_wq(layernorm(x, 2), wqa, Q3)

    def read_started(m):
        return jnp.where(m > SWITCH1, R_STEP * (m - SWITCH1) + R_BURST, 0)

    def wait_second_read():
        wait_for(slots(B_REST, 8 - N_KEPT), sem_b4.at[5])
        for grp, first in enumerate((8, 160, 168, 32)):
            wait_for(slots(first, 8), sem_b4.at[grp])
        wait_for(pool.at[pl.ds(40, 8), head_rows, :], sem_b4.at[4])

    def layer3(n):
        grp, j = ((n >> 2) + 2) & 7, n & 3
        k, v = a3_slots(grp)

        @pl.when((grp < 2) & (j == 0))
        def _():
            wait_for(slots(k, 16), sem_a3.at[2 * grp])
            wait_for(slots(v, 16), sem_a3.at[2 * grp + 1])

        def issue_point(i):
            m = 2 * n + i
            write_zeros(*(Z_LEAD + Z_STEP1 * jnp.minimum(t, SWITCH1) for t in (m, m + 1)))
            wait_zeros(0, jnp.where(m == SWITCH1, Z_FIRST - Z_OVERLAP, 0))
            issue(read_started(m), read_started(m + 1), second_read)
            _once_if(m == SWITCH2, wait_second_read)
            write_zeros(*(Z_FIRST + Z_STEP2 * jnp.maximum(t - SWITCH2, 0) for t in (m, m + 1)))
        a_head(_member(grp, j), k + 4 * j, v + 4 * j, (Q3, Q1), O3, C3_SLOTS,
               (P3_SLOT, P1_SLOT), issue_point)
    _loop(0, H, layer3)
    wait_for(pool.at[pl.ds(40, 8), tail_rows, :], sem_b4.at[6])

    z_next = [Z_FIRST + Z_STEP2 * (2 * H - SWITCH2)]

    def zeros_per_step(steps, units):
        lo = z_next[0]
        z_next[0] = lo + steps * units
        return lambda i: write_zeros(lo + units * i, lo + units * (i + 1))

    def zeros(units):
        zeros_per_step(1, units)(0)

    zeros(7)
    x = x + heads_wo(O3, woa)
    x_wq(layernorm(x, 3), wqb, Q4)
    zeros4 = zeros_per_step(8, 4)
    _loop(0, 8, lambda grp: b_group(
        grp, b4_slots(grp), (Q4, Q2), O4, ((AUX_SLOT, AUX_P4), (P2_SLOT, 0)),
        lambda: zeros4(grp)))
    zeros(7)
    io[0, 0] = (x + heads_wo(O4, wob)).astype(bf16)
    y_out = copy(io.at[0], out_hbm, sem_io.at[0])
    y_out.start()

    x_wo_t(row(G1 + 3), wob, DO_LATE)
    zeros4b = zeros_per_step(8, 4)

    def layer4_bwd(grp):
        def keep(j, h, ds):
            pool[AUX_SLOT, b_rows(AUX_DS4, h), :] = ds
        p = [pool[AUX_SLOT, b_rows(AUX_P4, _member(grp, j)), :] for j in range(4)]
        b_group_bwd(grp, p, DO_LATE, DQ4, keep, lambda: zeros4b(grp))
    _loop(0, 8, layer4_bwd)

    zeros(6)
    g = row(G1 + 3) + layernorm_bwd(heads_wq_t(DQ4, wqb), 3)
    rows[pl.ds(G1 + 2, 1), :] = g
    x_wo_t(g, woa, DQ3)
    zeros(6)
    a_dq(DQ3, DQ3, C3_SLOTS)
    g = g + layernorm_bwd(heads_wq_t(DQ3, wqa), 2)
    rows[pl.ds(G1 + 1, 1), :] = g

    zeros(12)
    x_wo_t(g, wob, DO_EARLY)
    dwo(wob, dbwo, sem_w.at[3], 1, 3, O2, O4)
    zeros2b = zeros_per_step(8, 2)

    def layer2_bwd(grp):
        p = [pool[P2_SLOT, b_rows(0, _member(grp, j)), :] for j in range(4)]
        pad = jnp.zeros((96, 128), bf16)

        def keep(j, h, ds):
            pool[AUX_SLOT, coef_rows(0, j), :] = jnp.concatenate(
                [p[j], pool[AUX_SLOT, b_rows(AUX_P4, h), :], pad], axis=0).T
            pool[AUX_SLOT, coef_rows(1, j), :] = jnp.concatenate(
                [ds, pool[AUX_SLOT, b_rows(AUX_DS4, h), :], pad], axis=0).T
        b_group_bwd(grp, p, DO_EARLY, DQ_EARLY, keep, lambda: zeros2b(grp))
        emit(grp, grp, SK - WIN, ((dbv, DO_EARLY, DO_LATE), (dbk, Q2, Q4)), 16, 0)
    _loop(0, 8, layer2_bwd)

    zeros(5)
    g = g + layernorm_bwd(heads_wq_t(DQ_EARLY, wqb), 1)
    rows[pl.ds(G1, 1), :] = g
    dwq(wqb, dbwq, sem_w.at[2], 1, 3, DQ_EARLY, DQ4)

    zeros(4)
    x_wo_t(row(G1 + 2), woa, DO_LATE)
    x_wo_t(g, woa, DO_EARLY)
    dwo(woa, dawo, sem_w.at[1], 0, 2, O1, O3)
    zeros(4)
    assert z_next[0] == Z_UNITS
    a_dq(DO_EARLY, DQ_EARLY, C1_SLOTS)
    io[1, 0] = (g + layernorm_bwd(heads_wq_t(DQ_EARLY, wqa), 0)).astype(bf16)
    dx_out = copy(io.at[1], dx_hbm, sem_io.at[1])
    dx_out.start()
    dwq(wqa, dawq, sem_w.at[0], 0, 2, DQ_EARLY, DQ3)

    def cache_grads(grp):
        def coefficients(j):
            h = _member(grp, j)
            vslot = a3_slots(grp)[1] + 4 * j
            lhs = _diag(head_vec(DO_EARLY, h), head_vec(DO_LATE, h))
            dp = [blk for c in range(4) for blk in against_rows(lhs, vslot + c)]
            p = [pool[slot, p_rows(h), :] for slot in (P1_SLOT, P3_SLOT)]
            ds = [_softmax_bwd(p[l].astype(f32), _pick(dp, l)) for l in range(2)]
            pool[AUX_SLOT, coef_rows(0, j), :] = jnp.concatenate(p, axis=0).T
            pool[AUX_SLOT, coef_rows(1, j), :] = jnp.concatenate(ds, axis=0).astype(bf16).T
        _loop(0, 4, coefficients)
        _loop(0, 4, lambda c: emit(
            8 + 4 * grp + c, grp, CH * c, ((dav, DO_EARLY, DO_LATE), (dak, Q1, Q3)), 64, 16 * c))
    _loop(0, 8, cache_grads)

    y_out.wait()
    dx_out.wait()
    wait_zeros(Z_FIRST - Z_OVERLAP, Z_UNITS)
    for i, buf in enumerate((wqa, woa, wqb, wob)):
        wait_for(buf, sem_w.at[i])
    for b in range(NSTAGE):
        wait_stage(b)


@jax.jit
def pallas_interleave_layers__gqa_block_cached__sliding_block_cached__decode_kernel(
    A_x: jax.Array,
    A_k_cache: jax.Array,
    A_v_cache: jax.Array,
    A_wq: jax.Array,
    A_wo: jax.Array,
    B_x: jax.Array,
    B_k_cache: jax.Array,
    B_v_cache: jax.Array,
    B_wq: jax.Array,
    B_wo: jax.Array,
    grad_out: jax.Array,
):
    del B_x
    weights = (A_k_cache, A_v_cache, A_wq, A_wo, B_k_cache, B_v_cache, B_wq, B_wo)
    views = [w.reshape(shape) for w, shape in
             zip(weights, (CACHE_VIEW, CACHE_VIEW, WQ_VIEW, WO_VIEW) * 2)]
    hbm = pl.BlockSpec(memory_space=pl.ANY)
    dma = pltpu.SemaphoreType.DMA
    outs = pl.pallas_call(
        _kernel,
        out_shape=[jax.ShapeDtypeStruct(a.shape, a.dtype) for a in [A_x, A_x] + views],
        in_specs=[hbm] * 10,
        out_specs=[hbm] * 10,
        scratch_shapes=[
            pltpu.VMEM((NSLOT, CH, DH), bf16),
            pltpu.VMEM((2, 5, D // 5, H * DH // 2), bf16),
            pltpu.VMEM(WO_VIEW, bf16),
            pltpu.VMEM((2, 5, D // 5, H * DH // 2), bf16),
            pltpu.VMEM(WO_VIEW, bf16),
            pltpu.VMEM((4, RUN, DH), bf16),
            pltpu.VMEM((NVEC, H, DH), f32),
            pltpu.VMEM((8, D), f32),
            pltpu.VMEM((8, 128), f32),
            pltpu.VMEM((2, 1, 1, D), bf16),
            dma((8,)), dma((4,)), dma((17,)), dma((7,)), dma((4,)), dma((2,)),
            dma((NSTAGE,)), dma((2,)),
        ],
        compiler_params=pltpu.CompilerParams(
            vmem_limit_bytes=128 * 1024 * 1024,
            disable_bounds_checks=True,
            disable_semaphore_checks=True,
        ),
    )(A_x, *views, grad_out)
    return tuple(o.reshape(a.shape) for o, a in zip(outs, (A_x, A_x) + weights))
```
